```python
import os as _os
_os.environ.setdefault('JAX_PLATFORMS', 'cpu')
import jax
import jax.numpy as jnp

def _softmax(x, axis=-1):
    return jax.nn.softmax(x, axis=axis)

def _gelu(x):
    return jax.nn.gelu(x, approximate=True)

def _silu(x):
    return jax.nn.silu(x)

def _sigmoid(x):
    return jax.nn.sigmoid(x)

def _layernorm(x, axis=-1, eps=1e-05):
    m = jnp.mean(x, axis=axis, keepdims=True)
    v = jnp.var(x, axis=axis, keepdims=True)
    return (x - m) / jnp.sqrt(v + eps)

def _scatter_add(tgt, idx, src, axis=0):
    return tgt.at[idx].add(src)

def _segment_sum(src, seg, n):
    return jax.ops.segment_sum(src, seg, n)

class _Rng:

    def __init__(self, key):
        self._k = key

    def _next(self):
        self._k, sub = jax.random.split(self._k)
        return sub

    def normal(self, shape):
        return jax.random.normal(self._next(), shape, dtype=jnp.bfloat16)

    def randint(self, lo, hi, shape):
        return jax.random.randint(self._next(), shape, lo, hi, dtype=jnp.int32)

    def uniform(self, shape, lo=0.0, hi=1.0):
        return jax.random.uniform(self._next(), shape, jnp.bfloat16, lo, hi)

    def permutation(self, n):
        return jax.random.permutation(self._next(), n)
kernel_name = 'standalone__conformer_family_e_branchformer__speech'

def setup_inputs():
    _rng = _Rng(jax.random.key(int.from_bytes(__import__("os").urandom(4), "little")))
    _w = lambda a: (lambda t: t.astype(jnp.bfloat16) if jnp.issubdtype(t.dtype, jnp.floating) else t)(jnp.asarray(a))
    B, T, D, K = (2, 4000, 512, 5)
    return {'x': _w((lambda *s: _rng.normal(s) * 0.05)(B, T, D)), 'w_qkv': _w((lambda *s: _rng.normal(s) * 0.05)(D, 3 * D)), 'w_att_out': _w((lambda *s: _rng.normal(s) * 0.05)(D, D)), 'w_mlp_in': _w((lambda *s: _rng.normal(s) * 0.05)(D, 2 * D)), 'dw_csgu': _w((lambda *s: _rng.normal(s) * 0.05)(K, D)), 'w_mlp_out': _w((lambda *s: _rng.normal(s) * 0.05)(D, D)), 'dw_merge': _w((lambda *s: _rng.normal(s) * 0.05)(K, 2 * D)), 'w_merge': _w((lambda *s: _rng.normal(s) * 0.05)(2 * D, D))}

def reference(x, w_qkv, w_att_out, w_mlp_in, dw_csgu, w_mlp_out, dw_merge, w_merge):
    B, T, D = x.shape
    K = dw_csgu.shape[0]
    pad = K // 2
    xa = _layernorm(x, axis=-1)
    qkv = jnp.einsum('btd,de->bte', xa, w_qkv)
    q, k, v = (qkv[..., :D].copy(), qkv[..., D:2 * D].copy(), qkv[..., 2 * D:].copy())
    scores = jnp.einsum('btd,bsd->bts', q, k) * D ** (-0.5)
    p = _softmax(scores, axis=-1)
    attn = jnp.einsum('bts,bsd->btd', p, v)
    glob = jnp.einsum('btd,de->bte', attn, w_att_out)
    xc = _layernorm(x, axis=-1)
    h = _gelu(jnp.einsum('btd,de->bte', xc, w_mlp_in))
    u, g = (h[..., :D].copy(), h[..., D:].copy())
    g = _layernorm(g, axis=-1)
    gp = jnp.pad(g, ((0, 0), (pad, pad), (0, 0)))
    gc = jnp.zeros_like(g)
    for i in range(K):
        gc = gc + gp[:, i:i + T, :] * dw_csgu[i][None, None, :]
    loc = jnp.einsum('btd,de->bte', u * gc, w_mlp_out)
    m = jnp.concatenate([glob, loc], axis=-1)
    mp = jnp.pad(m, ((0, 0), (pad, pad), (0, 0)))
    mc = jnp.zeros_like(m)
    for i in range(K):
        mc = mc + mp[:, i:i + T, :] * dw_merge[i][None, None, :]
    m = m + mc
    return x + jnp.einsum('btc,cd->btd', m, w_merge)
```

```python
import functools
import jax
import jax.numpy as jnp
from jax import lax
import jax.experimental.pallas as pl
import jax.experimental.pallas.tpu as pltpu

F32 = jnp.float32
BF16 = jnp.bfloat16
U32 = jnp.uint32
LOG2E = 1.4426950408889634
NT_DIMS = (((1,), (1,)), ((), ()))
NEG = -1e30


def _ln(xf, eps=1e-5):
    mu = jnp.mean(xf, axis=-1, keepdims=True)
    xc = xf - mu
    var = jnp.mean(xc * xc, axis=-1, keepdims=True)
    return xc * lax.rsqrt(var + eps)


def _gelu(x):
    c0 = 0.7978845608028654
    c1 = 0.7978845608028654 * 0.044715
    inner = x * (c0 + c1 * (x * x))
    hx = 0.5 * x
    return hx + hx * jnp.tanh(inner)


def _dot(a, b):
    return jnp.dot(a, b, preferred_element_type=F32)


def _dot_nt(a, b):
    return lax.dot_general(a, b, NT_DIMS, preferred_element_type=F32)


def _lhs_f32(a11, a12, a21, a22):
    return [a11 + a22, a21 + a22, a11, a22, a11 + a12, a21 - a11, a12 - a22]


def _lhs_combos(a11, a12, a21, a22):
    return [v.astype(BF16) for v in _lhs_f32(a11, a12, a21, a22)]


def _rhs_combos(b11, b12, b21, b22):
    return [b11 + b22, b11, b12 - b22, b21 - b11, b22, b11 + b12, b21 + b22]


def _out_combos(m1, m2, m3, m4, m5, m6, m7):
    return m1 + m4 - m5 + m7, m3 + m5, m2 + m4, m1 - m2 + m3 + m6


def _split4(a):
    r, c = a.shape
    h, w = r // 2, c // 2
    return a[:h, :w], a[:h, w:], a[h:, :w], a[h:, w:]


def _pk(v):
    return pltpu.bitcast(v, U32)


def _upk(v):
    return pltpu.bitcast(v, BF16)


def _vregs(v):
    b = pltpu.bitcast(v, U32)
    r, c = b.shape
    return [b[i:i + 8, j:j + 128] for i in range(0, r, 8) for j in range(0, c, 128)]


def _token(vals):
    tiles = []
    for v in vals:
        tiles += _vregs(v)
    return functools.reduce(jnp.bitwise_or, tiles)


@jax.jit
def pallas_standalone__conformer_family_e_branchformer__speech_kernel(
    x, w_qkv, w_att_out, w_mlp_in, dw_csgu, w_mlp_out, dw_merge, w_merge):
    B, T, D = x.shape
    KW = dw_csgu.shape[0]
    assert KW == 5 and B == 2
    TQ = 448
    H = TQ // 2
    HD = D // 2
    NT = pl.cdiv(T, TQ)
    PAD = 16
    HE = (TQ + 2 * PAD) // 2
    S = 4096
    SH = S // 2
    W = 512
    NCH = SH // W
    LC = 256
    NLC = SH // LC
    XR = PAD + S + PAD
    MR = PAD + NT * TQ + PAD
    NC = D // 128
    NTT = B * NT
    NSTEPS = NTT + 2
    scale = float(D) ** -0.5 * LOG2E
    RB = 16

    def kernel(x_hbm, wqkv_hbm, wo_hbm, win_hbm, dwc_ref, wout_hbm, dwm_ref, wm_hbm,
               o_ref,
               x_ref, wqkv_ref, wo_ref, win_ref, wout_ref, wm_ref,
               xa_ref, kc_ref, kn_ref, a7, wu7, wg7, wout7, wvo7, wm7,
               cwc_ref, cwm_ref,
               s_ref, xa7, xe7, q7, y7, z7, ml7, u_ref, g_ref, m_ref,
               sems):
        s = pl.program_id(0)
        zs = s >> 30
        zero = jnp.full((8, 128), zs, jnp.int32).astype(U32)

        def ln_rows(kdst, sb, db, c, r, n):
            rl = pl.multiple_of(c * LC + r, 16)
            rr = pl.multiple_of(SH + c * LC + r, 16)
            xl = _ln(x_ref[sb, pl.ds(rl, n), :].astype(F32))
            xr = _ln(x_ref[sb, pl.ds(rr, n), :].astype(F32))
            l1, l2, r1, r2 = xl[:, :HD], xl[:, HD:], xr[:, :HD], xr[:, HD:]
            hl = pl.multiple_of((c * LC + r) // 2, 8)
            xa_ref[db, pl.ds(PAD // 2 + hl, n // 2), :] = _pk(xl.astype(BF16))
            xa_ref[db, pl.ds((PAD + SH) // 2 + hl, n // 2), :] = _pk(xr.astype(BF16))
            for k, v in enumerate([l1 + r2, l1, r1 - r2, l2 - l1, r2, l1 + r1, l2 + r2]):
                kdst[k, pl.ds(hl, n // 2), :] = _pk(v.astype(BF16))
            return []

        def lhs_tile_piece(dst, b, row0, half, r):
            top = _upk(xa_ref[b, pl.ds(pl.multiple_of((row0 + r) // 2, 8), RB // 2), :])
            bot = _upk(xa_ref[b, pl.ds(pl.multiple_of((row0 + half + r) // 2, 8), RB // 2), :])
            tf, bf = top.astype(F32), bot.astype(F32)
            a11, a12, a21, a22 = tf[:, :HD], tf[:, HD:], bf[:, :HD], bf[:, HD:]
            vals = [(a11 + a22).astype(BF16), (a21 + a22).astype(BF16), top[:, :HD], bot[:, HD:],
                    (a11 + a12).astype(BF16), (a21 - a11).astype(BF16), (a12 - a22).astype(BF16)]
            for k, v in enumerate(vals):
                dst[k, r // 2:(r + RB) // 2, :] = _pk(v)
            return []

        def next_lhs_pieces(sn):
            bn = sn // NT
            t0n = (sn % NT) * TQ
            ps = [functools.partial(lhs_tile_piece, xa7, bn, PAD + t0n, H, r) for r in range(0, H, RB)]
            ps += [functools.partial(lhs_tile_piece, xe7, bn, t0n, HE, r) for r in range(0, HE, RB)]
            return ps

        def copies():
            return [
                pltpu.make_async_copy(wqkv_hbm, wqkv_ref, sems.at[0]),
                pltpu.make_async_copy(x_hbm.at[0], x_ref.at[0, pl.ds(0, T), :], sems.at[1]),
                pltpu.make_async_copy(wo_hbm, wo_ref, sems.at[2]),
                pltpu.make_async_copy(win_hbm, win_ref, sems.at[3]),
                pltpu.make_async_copy(wout_hbm, wout_ref, sems.at[4]),
                pltpu.make_async_copy(wm_hbm, wm_ref, sems.at[5]),
            ]

        def x1_copy():
            return pltpu.make_async_copy(x_hbm.at[1], x_ref.at[1, pl.ds(0, T), :], sems.at[6])

        def set_w7(dst, w):
            for k, v in enumerate(_rhs_combos(*_split4(w))):
                dst[k] = _pk(v.astype(BF16))

        @pl.when(s == 0)
        def _prologue():
            cps = copies()
            for cp in cps:
                cp.start()
            x1_copy().start()
            for b in range(B):
                x_ref[b, T:S, :] = jnp.zeros((S - T, D), BF16)
                xa_ref[b, 0:PAD // 2, :] = jnp.zeros((PAD // 2, D), U32)
                xa_ref[b, (PAD + S) // 2:XR // 2, :] = jnp.zeros((PAD // 2, D), U32)
            for c in range(2 * NC):
                m_ref[c, 0:TQ + 2 * PAD, :] = jnp.zeros((TQ + 2 * PAD, 128), F32)
                m_ref[c, MR - PAD:MR, :] = jnp.zeros((PAD, 128), F32)
            for d in range(KW):
                cwc_ref[d] = jnp.broadcast_to(dwc_ref[d:d + 1, :].astype(F32), (8, D))
                w = dwm_ref[d:d + 1, :].astype(F32)
                if d == KW // 2:
                    w = w + 1.0
                cwm_ref[d] = jnp.broadcast_to(w, (8, 2 * D))
            y7[...] = jnp.zeros(y7.shape, U32)
            cps[0].wait()
            set_w7(a7, _dot_nt(wqkv_ref[:, 0:D], wqkv_ref[:, D:2 * D]) * scale)
            cps[1].wait()

            def body(c, carry):
                for r in range(0, LC, 64):
                    ln_rows(kc_ref, 0, 0, c, r, 64)
                return carry
            lax.fori_loop(0, NLC, body, 0)
            for p in next_lhs_pieces(0):
                p()
            cps[2].wait()
            set_w7(wvo7, _dot(wqkv_ref[:, 2 * D:3 * D], wo_ref[...]))
            cps[3].wait()
            set_w7(wu7, win_ref[:, 0:D].astype(F32))
            set_w7(wg7, win_ref[:, D:2 * D].astype(F32))
            cps[4].wait()
            set_w7(wout7, wout_ref[...].astype(F32))
            cps[5].wait()
            set_w7(wm7, wm_ref[...].astype(F32))

        @pl.when(s == 1)
        def _():
            x1_copy().wait()

        @pl.when(s == NT)
        def _():
            def body(j, carry):
                r = pl.multiple_of(j * 64, 64)
                for k in range(7):
                    kc_ref[k, pl.ds(r, 64), :] = kn_ref[k, pl.ds(r, 64), :]
                return carry
            lax.fori_loop(0, SH // 2 // 64, body, 0)

        def tied(lhs, toks):
            if not toks:
                return lhs
            t = functools.reduce(jnp.bitwise_or, toks) & zero
            head = pltpu.bitcast(pltpu.bitcast(lhs[:16, :128], U32) | t, BF16)
            return jnp.concatenate(
                [jnp.concatenate([head, lhs[:16, 128:]], axis=1), lhs[16:]], axis=0)

        def mm_units(lhs_ref, w_ref, out):
            def unit(k, toks):
                out[k] = _dot(tied(_upk(lhs_ref[k]), toks), _upk(w_ref[k]))
            return [functools.partial(unit, k) for k in range(7)]

        def oc(ms, r, n=RB):
            return _out_combos(*[m[r:r + n, :] for m in ms])

        def store_m_pieces(c0, r0, t0, ms):
            def piece(r):
                blocks = oc(ms, r)
                row = lax.broadcasted_iota(jnp.int32, (RB, 128), 0)
                outs = []
                for half in range(2):
                    valid = (row + (t0 + half * H + r)) < T
                    for cb in range(2):
                        blk = blocks[2 * half + cb]
                        for k in range(HD // 128):
                            v = jnp.where(valid, blk[:, k * 128:(k + 1) * 128], 0.0)
                            m_ref[c0 + cb * (HD // 128) + k,
                                  pl.ds(pl.multiple_of(r0 + half * H + r, 8), RB), :] = v
                return []
            return [functools.partial(piece, r) for r in range(0, H, RB)]

        def conv_block(ref, cw_ref, c, r, n):
            acc = None
            for d in range(KW):
                w = cw_ref[d, :, c * 128:(c + 1) * 128]
                v = ref[c, PAD - 2 + d + r:PAD - 2 + d + r + n, :].reshape(n // 8, 8, 128) * w[None]
                acc = v if acc is None else acc + v
            return acc.reshape(n, 128)

        def glob_work():
            sp = jnp.maximum(s - 1, 0)
            i = sp % NT
            ms = [None] * 7
            return mm_units(y7, wvo7, ms), store_m_pieces(0, PAD + i * TQ, i * TQ, ms)

        def merge_lhs_pieces():
            jg = jnp.maximum(s - 2, 0)
            base = pl.multiple_of((jg % NT) * TQ, 16)
            win = m_ref.at[:, pl.ds(base, TQ + 2 * PAD), :]

            def piece(c, r):
                a11 = conv_block(win, cwm_ref, c, r, RB)
                a21 = conv_block(win, cwm_ref, c, H + r, RB)
                a12 = conv_block(win, cwm_ref, NC + c, r, RB)
                a22 = conv_block(win, cwm_ref, NC + c, H + r, RB)
                vals = _lhs_combos(a11, a12, a21, a22)
                for k, v in enumerate(vals):
                    ml7[k, r // 2:(r + RB) // 2, c * 128:(c + 1) * 128] = _pk(v)
                return [a11 + a22, a12 + a21]
            return [functools.partial(piece, c, r) for r in range(0, H, RB) for c in range(NC)]

        def merge_work():
            jg = jnp.maximum(s - 2, 0)
            b = jg // NT
            base = (jg % NT) * TQ
            ms = [None] * 7

            def piece(r):
                c11, c12, c21, c22 = oc(ms, r)
                outs = []
                for half, (lo, hi) in enumerate(((c11, c12), (c21, c22))):
                    xr = x_ref[b, pl.ds(pl.multiple_of(base + half * H + r, 16), RB), :].astype(F32)
                    v = (xr + jnp.concatenate([lo, hi], axis=1)).astype(o_ref.dtype)
                    o_ref[0, half * H + r:half * H + r + RB, :] = v
                return []
            return mm_units(ml7, wm7, ms), [functools.partial(piece, r) for r in range(0, H, RB)]

        def run(units, plan):
            for i, u in enumerate(units):
                toks = []
                for p in plan.get(i, []):
                    vals = p()
                    if vals:
                        toks.append(_token(vals))
                u(toks)

        def spread(plan, pieces, lo, hi):
            n = hi - lo + 1
            for j, p in enumerate(pieces):
                plan.setdefault(lo + (j * n) // len(pieces), []).append(p)

        def main_step():
            b = s // NT
            i = s % NT
            t0 = i * TQ
            r0 = pl.multiple_of(PAD + t0, 16)

            g_units, g_pieces = glob_work()
            qm, um, gm = [None] * 7, [None] * 7, [None] * 7

            def q_piece(r):
                vals = _lhs_combos(*oc(qm, r))
                for k, v in enumerate(vals):
                    q7[k, r // 2:(r + RB) // 2, :] = _pk(v)
                return []

            def u_piece(r):
                c11, c12, c21, c22 = [_gelu(v) for v in oc(um, r)]
                u_ref[r:r + RB, 0:HD] = c11
                u_ref[r:r + RB, HD:D] = c12
                u_ref[H + r:H + r + RB, 0:HD] = c21
                u_ref[H + r:H + r + RB, HD:D] = c22
                return [(c11 + c12) + (c21 + c22)]

            def gt_piece(r, half):
                blocks = oc(gm, r)
                g = _ln(_gelu(jnp.concatenate(blocks[2 * half:2 * half + 2], axis=1)))
                trow = lax.broadcasted_iota(jnp.int32, (RB, 128), 0) + (t0 - PAD + half * HE + r)
                valid = (trow >= 0) & (trow < T)
                outs = []
                for c in range(NC):
                    v = jnp.where(valid, g[:, c * 128:(c + 1) * 128], 0.0)
                    g_ref[c, half * HE + r:half * HE + r + RB, :] = v
                    outs.append(v)
                return outs

            def kop(k, sl):
                return _upk(kc_ref[k, sl.start // 2:sl.stop // 2, :])

            km = [[None] * 7 for _ in range(NCH)]

            def k_units(c):
                sl = slice(c * W, (c + 1) * W)

                def unit(k, toks):
                    km[c][k] = _dot_nt(tied(_upk(q7[k]), toks), kop(k, sl))
                return [functools.partial(unit, k) for k in range(7)]

            SRB = 8
            stat = {}

            def k_piece(c, r):
                sl = slice(c * W, (c + 1) * W)
                c11, c12, c21, c22 = oc(km[c], r, SRB)
                if SH + (c + 1) * W > T:
                    col = lax.broadcasted_iota(jnp.int32, (SRB, W), 1)
                    ok = col < (T - SH - c * W)
                    c12 = jnp.where(ok, c12, NEG)
                    c22 = jnp.where(ok, c22, NEG)
                for idx, v in enumerate((c11, c12, c21, c22)):
                    s_ref[idx + zs, r:r + SRB, sl] = v
                outs = []
                for h, (a, bb) in enumerate(((c11, c12), (c21, c22))):
                    tiles = [v[:, k * 128:(k + 1) * 128] for v in (a, bb) for k in range(W // 128)]
                    cm = functools.reduce(jnp.maximum, tiles)
                    l = functools.reduce(jnp.add, [jnp.exp2(t - cm) for t in tiles])
                    stat[c, h, r] = (cm, l)
                    outs.append(l)
                return outs

            def k_pieces(c):
                return [functools.partial(k_piece, c, r) for r in range(0, H, SRB)]

            def fin(h):
                ms = [jnp.concatenate([stat[c, h, r][0] for r in range(0, H, SRB)], axis=0) for c in range(NCH)]
                ls = [jnp.concatenate([stat[c, h, r][1] for r in range(0, H, SRB)], axis=0) for c in range(NCH)]
                m = jnp.max(functools.reduce(jnp.maximum, ms), axis=1, keepdims=True)
                l = functools.reduce(jnp.add, [ls[c] * jnp.exp2(ms[c] - m) for c in range(NCH)])
                return m + jnp.log2(jnp.sum(l, axis=1, keepdims=True))

            lb = jnp.where((s >= 1) & (s < NT), 1, 0)
            db = jnp.where(s < NT, 1, 0)
            lc = jnp.where(s < NT, jnp.maximum(s - 1, 0), (s - NT) % NLC)
            ln_pieces = [functools.partial(ln_rows, kn_ref, lb, db, lc, r, RB) for r in range(0, LC, RB)]

            n = [None] * 7
            tmap = [0, 6, 1, 4, 5, 3, 2]
            off = []

            def p_units(c):
                sl = slice(c * W, (c + 1) * W)
                cache = {}

                def lhs(k):
                    if not off:
                        off.extend([fin(0), fin(1)])
                    if not cache:
                        cache['p'] = [jnp.exp2(s_ref[idx + zs, :, sl] - off[idx // 2]) for idx in range(4)]
                    p11, p12, p21, p22 = cache['p']
                    return [lambda: p11 + p22, lambda: p11, lambda: p21 - p22, lambda: p12 - p11,
                            lambda: p22, lambda: p11 + p21, lambda: p12 + p22][k]()

                def unit(k, toks):
                    r = _dot(tied(lhs(k).astype(BF16), toks), kop(tmap[k], sl))
                    n[k] = r if n[k] is None else n[k] + r
                return [functools.partial(unit, k) for k in range(7)]

            def z_piece(c, r):
                vals = []
                for cc in (c, c + NC // 2):
                    for half in range(2):
                        rr = half * H + r
                        gc = conv_block(g_ref, cwc_ref, cc, rr, RB)
                        vals.append(u_ref[rr:rr + RB, cc * 128:(cc + 1) * 128] * gc)
                a11, a21, a12, a22 = vals
                outs = _lhs_combos(a11, a12, a21, a22)
                for k, v in enumerate(outs):
                    z7[k, r // 2:(r + RB) // 2, c * 128:(c + 1) * 128] = _pk(v)
                return [a11 + a22, a12 + a21]
            z_pieces = [functools.partial(z_piece, c, r) for r in range(0, H, RB) for c in range(NC // 2)]

            def y_piece(r):
                n1, n2, n3, n4, n5, n6, n7 = [v[r:r + RB, :] for v in n]
                y11 = n1 + n4 - n5 + n7
                y21 = n3 + n5
                y12 = n2 + n4
                y22 = n1 - n2 + n3 + n6
                outs = _lhs_combos(y11, y12, y21, y22)
                for k, v in enumerate(outs):
                    y7[k, r // 2:(r + RB) // 2, :] = _pk(v)
                return []

            lm = [None] * 7
            mg_units, mg_pieces = merge_work()
            units = (mm_units(xa7, a7, qm) + mm_units(xa7, wu7, um) + mm_units(xe7, wg7, gm)
                     + k_units(0) + g_units + k_units(1) + k_units(2) + k_units(3) + mg_units
                     + p_units(0) + p_units(1) + p_units(2) + p_units(3) + mm_units(z7, wout7, lm))
            Q, U, TT, K0, G, K1, K2, K3, MG, P0, L = 0, 7, 14, 21, 28, 35, 42, 49, 56, 63, 91
            plan = {}
            spread(plan, [functools.partial(q_piece, r) for r in range(0, H, RB)], U + 2, TT + 1)
            spread(plan, [functools.partial(u_piece, r) for r in range(0, H, RB)], TT + 2, K0 + 2)
            spread(plan, [functools.partial(gt_piece, r, h) for h in range(2) for r in range(0, HE, RB)],
                   K0 + 1, K1 + 3)
            spread(plan, k_pieces(0), G + 1, K1 + 6)
            spread(plan, g_pieces, K1 + 1, K1 + 3)
            spread(plan, merge_lhs_pieces(), K1 + 4, MG)
            spread(plan, k_pieces(1), K2 + 1, K3)
            spread(plan, k_pieces(2), K3 + 1, MG)
            spread(plan, k_pieces(3), MG + 1, MG + 4)
            spread(plan, mg_pieces, P0 + 2, P0 + 8)
            spread(plan, ln_pieces, P0 + 1, P0 + 27)
            spread(plan, z_pieces, P0 + 7, P0 + 27)
            spread(plan, next_lhs_pieces(jnp.minimum(s + 1, NTT - 1)), P0 + 1, P0 + 27)
            spread(plan, [functools.partial(y_piece, r) for r in range(0, H, RB)], L + 2, L + 6)
            run(units, plan)
            for p in store_m_pieces(NC, r0, t0, lm):
                p()

        @pl.when(s < NTT)
        def _():
            main_step()

        @pl.when(s >= NTT)
        def _():
            g_units, g_pieces = glob_work()
            run(g_units, {})
            for p in g_pieces:
                p()
            for p in merge_lhs_pieces():
                p()
            mg_units, mg_pieces = merge_work()
            run(mg_units, {})
            for p in mg_pieces:
                p()

    anyspec = pl.BlockSpec(memory_space=pl.ANY)

    def full(shape):
        return pl.BlockSpec(shape, lambda s: (0,) * len(shape))

    def out_map(s):
        jg = jnp.clip(s - 2, 0, NTT - 1)
        return (jg // NT, jg % NT, 0)

    return pl.pallas_call(
        kernel,
        grid=(NSTEPS,),
        in_specs=[anyspec, anyspec, anyspec, anyspec, full(dw_csgu.shape), anyspec,
                  full(dw_merge.shape), anyspec],
        out_specs=pl.BlockSpec((1, TQ, D), out_map),
        out_shape=jax.ShapeDtypeStruct((B, T, D), x.dtype),
        scratch_shapes=[
            pltpu.VMEM((B, S, D), BF16),
            pltpu.VMEM((D, 3 * D), BF16),
            pltpu.VMEM((D, D), BF16),
            pltpu.VMEM((D, 2 * D), BF16),
            pltpu.VMEM((D, D), BF16),
            pltpu.VMEM((2 * D, D), BF16),
            pltpu.VMEM((B, XR // 2, D), U32),
            pltpu.VMEM((7, SH // 2, HD), U32),
            pltpu.VMEM((7, SH // 2, HD), U32),
            pltpu.VMEM((7, HD // 2, HD), U32),
            pltpu.VMEM((7, HD // 2, HD), U32),
            pltpu.VMEM((7, HD // 2, HD), U32),
            pltpu.VMEM((7, HD // 2, HD), U32),
            pltpu.VMEM((7, HD // 2, HD), U32),
            pltpu.VMEM((7, D // 2, HD), U32),
            pltpu.VMEM((KW, 8, D), F32),
            pltpu.VMEM((KW, 8, 2 * D), F32),
            pltpu.VMEM((4, H, SH), F32),
            pltpu.VMEM((7, H // 2, HD), U32),
            pltpu.VMEM((7, HE // 2, HD), U32),
            pltpu.VMEM((7, H // 2, HD), U32),
            pltpu.VMEM((7, H // 2, HD), U32),
            pltpu.VMEM((7, H // 2, HD), U32),
            pltpu.VMEM((7, H // 2, D), U32),
            pltpu.VMEM((TQ, D), F32),
            pltpu.VMEM((NC, TQ + 2 * PAD, 128), F32),
            pltpu.VMEM((2 * NC, MR, 128), F32),
            pltpu.SemaphoreType.DMA((7,)),
        ],
        compiler_params=pltpu.CompilerParams(
            dimension_semantics=("arbitrary",), vmem_limit_bytes=110 * 1024 * 1024),
    )(x, w_qkv, w_att_out, w_mlp_in, dw_csgu, w_mlp_out, dw_merge, w_merge)
```

```python
import functools
import jax
import jax.numpy as jnp
from jax import lax
import jax.experimental.pallas as pl
import jax.experimental.pallas.tpu as pltpu

F32 = jnp.float32
BF16 = jnp.bfloat16
U32 = jnp.uint32
LOG2E = 1.4426950408889634
NT_DIMS = (((1,), (1,)), ((), ()))
NEG = -1e30


def _ln(xf, eps=1e-5):
    mu = jnp.mean(xf, axis=-1, keepdims=True)
    xc = xf - mu
    var = jnp.mean(xc * xc, axis=-1, keepdims=True)
    return xc * lax.rsqrt(var + eps)


def _gelu(x):
    c0 = 0.7978845608028654
    c1 = 0.7978845608028654 * 0.044715
    inner = x * (c0 + c1 * (x * x))
    hx = 0.5 * x
    return hx + hx * jnp.tanh(inner)


def _dot(a, b):
    return jnp.dot(a, b, preferred_element_type=F32)


def _dot_nt(a, b):
    return lax.dot_general(a, b, NT_DIMS, preferred_element_type=F32)


def _lhs_f32(a11, a12, a21, a22):
    return [a11 + a22, a21 + a22, a11, a22, a11 + a12, a21 - a11, a12 - a22]


def _lhs_combos(a11, a12, a21, a22):
    return [v.astype(BF16) for v in _lhs_f32(a11, a12, a21, a22)]


def _rhs_combos(b11, b12, b21, b22):
    return [b11 + b22, b11, b12 - b22, b21 - b11, b22, b11 + b12, b21 + b22]


def _out_combos(m1, m2, m3, m4, m5, m6, m7):
    return m1 + m4 - m5 + m7, m3 + m5, m2 + m4, m1 - m2 + m3 + m6


def _split4(a):
    r, c = a.shape
    h, w = r // 2, c // 2
    return a[:h, :w], a[:h, w:], a[h:, :w], a[h:, w:]


def _pk(v):
    return pltpu.bitcast(v, U32)


def _upk(v):
    return pltpu.bitcast(v, BF16)


def _pk16(v):
    return pltpu.pack_elementwise([v[:8], v[8:]], packed_dtype=BF16)


def _upk16(w):
    lo = pltpu.unpack_elementwise(w, index=0, packed_dtype=BF16, unpacked_dtype=F32)
    hi = pltpu.unpack_elementwise(w, index=1, packed_dtype=BF16, unpacked_dtype=F32)
    return jnp.concatenate([lo, hi], axis=0)


def _token(vals):
    tiles = []
    for v in vals:
        b = pltpu.bitcast(v, U32)
        r, c = b.shape
        tiles += [b[i:i + 8, j:j + 128] for i in range(0, r, 8) for j in range(0, c, 128)]
    return functools.reduce(jnp.bitwise_or, tiles)


def _cat7(parts, rows, cols):
    return [jnp.concatenate(
        [jnp.concatenate([parts[r, c][k] for c in cols], axis=1) if len(cols) > 1 else parts[r, cols[0]][k]
         for r in rows], axis=0) for k in range(7)]


@jax.jit
def pallas_standalone__conformer_family_e_branchformer__speech_kernel(
    x, w_qkv, w_att_out, w_mlp_in, dw_csgu, w_mlp_out, dw_merge, w_merge):
    B, T, D = x.shape
    KW = dw_csgu.shape[0]
    assert KW == 5 and B == 2
    TQ = 448
    H = TQ // 2
    HD = D // 2
    NT = pl.cdiv(T, TQ)
    PAD = 16
    HE = (TQ + 2 * PAD) // 2
    S = 4096
    SH = S // 2
    W = 512
    NCH = SH // W
    LC = 256
    NLC = SH // LC
    XR = PAD + S + PAD
    MH = 2 * PAD
    MR = MH + TQ
    NC = D // 128
    NTT = B * NT
    NSTEPS = NTT + 1
    scale = float(D) ** -0.5 * LOG2E
    RB = 16
    ROWS = list(range(0, H, RB))
    ROWS_E = list(range(0, HE, RB))

    def kernel(x_hbm, wqkv_hbm, wo_hbm, win_hbm, dwc_ref, wout_hbm, dwm_ref, wm_hbm,
               o_hbm,
               ob_ref, x_ref, wqkv_ref, wo_ref, win_ref, wout_ref, wm_ref,
               xa_ref, kc_ref, kn_ref, a7, wu7, wg7, wout7, wvo7, wm7,
               cwc_ref, cwm_ref,
               s_ref, yb_ref, q7, z7, ml7, u_ref, g_ref, m_ref,
               sems, xsems, osems):
        s = pl.program_id(0)
        zs = s >> 30
        zero = jnp.full((8, 128), zs, jnp.int32).astype(U32)

        def ln_rows(kdst, sb, db, c, r, z=None):
            rl = pl.multiple_of(c * LC + r, 16)
            rr = pl.multiple_of(SH + c * LC + r, 16)
            xl = x_ref[sb, pl.ds(PAD + rl, RB), :].astype(F32)
            xr = x_ref[sb, pl.ds(PAD + rr, RB), :].astype(F32)
            if z is not None:
                z2 = jnp.concatenate([z, z], axis=0)
                xl = jnp.concatenate([xl[:, :128] + z2, xl[:, 128:]], axis=1)
                xr = jnp.concatenate([xr[:, :128] + z2, xr[:, 128:]], axis=1)
            xl = _ln(xl)
            xr = _ln(xr)
            l1, l2, r1, r2 = xl[:, :HD], xl[:, HD:], xr[:, :HD], xr[:, HD:]
            hl = pl.multiple_of((c * LC + r) // 2, 8)
            xa_ref[db, pl.ds(PAD // 2 + hl, 8), :] = _pk16(xl)
            xa_ref[db, pl.ds((PAD + SH) // 2 + hl, 8), :] = _pk16(xr)
            for k, v in enumerate([l1 + r2, l1, r1 - r2, l2 - l1, r2, l1 + r1, l2 + r2]):
                kdst[k, pl.ds(hl, 8), :] = _pk16(v)
            return [l1 + r1, l2 + r2]

        def w_copy(i):
            srcs = [(wqkv_hbm, wqkv_ref), (wo_hbm, wo_ref), (win_hbm, win_ref), (wout_hbm, wout_ref),
                    (wm_hbm, wm_ref)]
            return pltpu.make_async_copy(srcs[i][0], srcs[i][1], sems.at[i])

        def x0_copy(c, h, n=LC):
            r = h * SH + c * LC
            if not isinstance(r, int):
                r = pl.multiple_of(r, LC)
            return pltpu.make_async_copy(x_hbm.at[0, pl.ds(r, n), :], x_ref.at[0, pl.ds(PAD + r, n), :],
                                         xsems.at[2 * c + h])

        def x1_copy():
            return pltpu.make_async_copy(x_hbm.at[1], x_ref.at[1, pl.ds(PAD, T), :], sems.at[5])

        def set_w7(dst, w):
            for k, v in enumerate(_rhs_combos(*_split4(w))):
                dst[k] = _pk(v.astype(BF16))

        @pl.when(s == 0)
        def _prologue():
            NLAST = T - SH - (NLC - 1) * LC
            for c in range(NLC):
                x0_copy(c, 0).start()
                x0_copy(c, 1, LC if c < NLC - 1 else NLAST).start()
            w_copy(0).start()
            w_copy(1).start()
            w_copy(2).start()
            w_copy(3).start()
            for b in range(B):
                x_ref[b, 0:PAD, :] = jnp.zeros((PAD, D), BF16)
                x_ref[b, PAD + T:PAD + S, :] = jnp.zeros((S - T, D), BF16)
                xa_ref[b, 0:PAD // 2, :] = jnp.zeros((PAD // 2, D), U32)
                xa_ref[b, (PAD + S) // 2:XR // 2, :] = jnp.zeros((PAD // 2, D), U32)
            m_ref[...] = jnp.zeros(m_ref.shape, F32)
            for d in range(KW):
                cwc_ref[d] = jnp.broadcast_to(dwc_ref[d:d + 1, :].astype(F32), (8, D))
                w = dwm_ref[d:d + 1, :].astype(F32)
                if d == KW // 2:
                    w = w + 1.0
                cwm_ref[d] = jnp.broadcast_to(w, (8, 2 * D))
            yb_ref[...] = jnp.zeros(yb_ref.shape, F32)
            def ln_chunk0(c):
                for r in range(0, LC, RB):
                    ln_rows(kc_ref, 0, 0, c, r)

            def body(c, carry):
                x0_copy(c, 0).wait()
                x0_copy(c, 1).wait()
                ln_chunk0(c)
                return carry
            lax.fori_loop(0, NLC - 1, body, 0)
            x0_copy(NLC - 1, 0).wait()
            x0_copy(NLC - 1, 1, NLAST).wait()
            lax.fori_loop(NLC - 1, NLC, lambda c, carry: (ln_chunk0(c), carry)[1], 0)
            w_copy(0).wait()
            set_w7(a7, _dot_nt(wqkv_ref[:, 0:D], wqkv_ref[:, D:2 * D]) * scale)
            w_copy(1).wait()
            set_w7(wvo7, _dot(wqkv_ref[:, 2 * D:3 * D], wo_ref[...]))
            w_copy(4).start()
            x1_copy().start()
            w_copy(2).wait()
            set_w7(wu7, win_ref[:, 0:D].astype(F32))
            set_w7(wg7, win_ref[:, D:2 * D].astype(F32))
            w_copy(3).wait()
            set_w7(wout7, wout_ref[...].astype(F32))
            wm7[...] = jnp.zeros(wm7.shape, U32)

        @pl.when(s == 1)
        def _():
            x1_copy().wait()
            w_copy(4).wait()
            set_w7(wm7, wm_ref[...].astype(F32))

        @pl.when(s == NT)
        def _():
            def body(j, carry):
                r = pl.multiple_of(j * 64, 64)
                for k in range(7):
                    kc_ref[k, pl.ds(r, 64), :] = kn_ref[k, pl.ds(r, 64), :]
                return carry
            lax.fori_loop(0, SH // 2 // 64, body, 0)

        def tie_head(head_u32, toks):
            return head_u32 | (functools.reduce(jnp.bitwise_or, toks) & zero)

        def zero_after(v):
            return pltpu.bitcast(pltpu.bitcast(v[:8, :128], U32) & zero, F32)

        def tied(lhs, toks):
            if not toks:
                return lhs
            head = _upk(tie_head(_pk(lhs[:16, :128]), toks))
            return jnp.concatenate(
                [jnp.concatenate([head, lhs[:16, 128:]], axis=1), lhs[16:]], axis=0)

        def tied_f32(lhs, toks):
            if not toks:
                return lhs
            head = pltpu.bitcast(tie_head(pltpu.bitcast(lhs[:8, :128], U32), toks), F32)
            return jnp.concatenate(
                [jnp.concatenate([head, lhs[:8, 128:]], axis=1), lhs[8:]], axis=0)

        def mm_units(get_lhs7, w_ref, out):
            cache = {}

            def unit(k, toks):
                if not cache:
                    cache['l'] = get_lhs7()
                out[k] = _dot(tied_f32(cache['l'][k], toks).astype(BF16), _upk(w_ref[k]))
                return out[k]
            return [functools.partial(unit, k) for k in range(7)]

        def oc(ms, r, n=RB):
            return _out_combos(*[m[r:r + n, :] for m in ms])

        def store_m_pieces(c0, tile, ms):
            t0 = (tile % NT) * TQ

            def tail():
                keep = (tile % NT) > 0
                for c in range(c0, c0 + NC):
                    m_ref[c, 0:MH, :] = jnp.where(keep, m_ref[c, TQ:TQ + MH, :], 0.0)
                return []

            def piece(r):
                blocks = oc(ms, r)
                row = lax.broadcasted_iota(jnp.int32, (RB, 128), 0)
                for half in range(2):
                    valid = (row + (t0 + half * H + r)) < T
                    for cb in range(2):
                        blk = blocks[2 * half + cb]
                        for k in range(HD // 128):
                            rr = MH + half * H + r
                            m_ref[c0 + cb * (HD // 128) + k, rr:rr + RB, :] = (
                                jnp.where(valid, blk[:, k * 128:(k + 1) * 128], 0.0))
                return []
            return [tail] + [functools.partial(piece, r) for r in ROWS]

        def conv_eo(ref, cw_ref, c, r, z=None):
            ws = []
            for d in range(KW):
                w = cw_ref[d, :, c * 128:(c + 1) * 128]
                ws.append(w if z is None else w + z)
            res = []
            for par in range(2):
                acc = None
                for d in range(KW):
                    v = ref[c, pl.ds(PAD - 2 + d + r + par, 8, stride=2), :] * ws[d]
                    acc = v if acc is None else acc + v
                res.append(acc)
            return res

        def store_lhs_eo(dst, r, c, a11, a12, a21, a22):
            ev = _lhs_f32(a11[0], a12[0], a21[0], a22[0])
            od = _lhs_f32(a11[1], a12[1], a21[1], a22[1])
            for k in range(7):
                dst[k, r // 2:r // 2 + 8, c * 128:(c + 1) * 128] = pltpu.pack_elementwise(
                    [ev[k], od[k]], packed_dtype=BF16)

        def glob_work():
            ms = [None] * 7
            units = mm_units(lambda: _lhs_f32(*[yb_ref[q] for q in range(4)]), wvo7, ms)
            return units, store_m_pieces(0, jnp.maximum(s - 1, 0), ms)

        def merge_work():
            jg = jnp.maximum(s - 1, 0)
            b = jg // NT
            base = pl.multiple_of((jg % NT) * TQ, 16)
            slot = s % 2

            def lhs_piece(c, r, z=None):
                a11 = conv_eo(m_ref, cwm_ref, c, r, z)
                a21 = conv_eo(m_ref, cwm_ref, c, H + r, z)
                a12 = conv_eo(m_ref, cwm_ref, NC + c, r, z)
                a22 = conv_eo(m_ref, cwm_ref, NC + c, H + r, z)
                store_lhs_eo(ml7, r, c, a11, a12, a21, a22)
                return []
            lhs_pieces = [functools.partial(lhs_piece, c, r) for r in ROWS for c in range(NC)]
            ms = [None] * 7

            def unit(k, toks):
                ms[k] = _dot(tied(_upk(ml7[k]), toks), _upk(wm7[k]))
                return ms[k]

            def piece(r):
                c11, c12, c21, c22 = oc(ms, r)
                for half, (lo, hi) in enumerate(((c11, c12), (c21, c22))):
                    xr = x_ref[b, pl.ds(pl.multiple_of(base + half * H + r, 16), RB), :].astype(F32)
                    ob_ref[slot, half * H + r:half * H + r + RB, :] = (
                        xr + jnp.concatenate([lo, hi], axis=1)).astype(ob_ref.dtype)
                return []
            return (lhs_pieces, [functools.partial(unit, k) for k in range(7)],
                    [functools.partial(piece, r) for r in ROWS])

        def out_copy(step, kind):
            jg = step - 1
            b = jg // NT
            j = jg % NT
            slot = step % 2
            if kind == 0:
                src_, off, n = ob_ref.at[slot, pl.ds(PAD, TQ - PAD), :], 0, TQ - PAD
            elif kind == 1:
                src_, off, n = ob_ref.at[slot], pl.multiple_of(j * TQ - PAD, 16), TQ
            else:
                n = T - ((NT - 1) * TQ - PAD)
                src_, off = ob_ref.at[slot, pl.ds(0, n), :], (NT - 1) * TQ - PAD
            return pltpu.make_async_copy(src_, o_hbm.at[b, pl.ds(off, n), :], osems.at[slot])

        def for_out(step, fn):
            j = (step - 1) % NT
            for kind, cond in enumerate((j == 0, (j > 0) & (j < NT - 1), j == NT - 1)):
                @pl.when(cond)
                def _(kind=kind):
                    fn(out_copy(step, kind))

        def run(units, plan):
            outs = []
            for i, u in enumerate(units):
                toks = []
                for p, a in plan.get(i, []):
                    vals = p() if a is None else p(z=zero_after(outs[a]))
                    if vals:
                        toks.append(_token(vals))
                outs.append(u(toks))

        def spread(plan, pieces, lo, hi, lag=None):
            n = hi - lo + 1
            for j, p in enumerate(pieces):
                i = lo + (j * n) // len(pieces)
                plan.setdefault(i, []).append((p, None if lag is None else i - lag))

        def main_step():
            b = s // NT
            i = s % NT
            t0 = i * TQ
            r0 = pl.multiple_of(PAD + t0, 16)

            g_units, g_pieces = glob_work()
            qm, um, gm = [None] * 7, [None] * 7, [None] * 7

            def xa_rows(row0, n):
                base = pl.multiple_of(row0 // 2, 8)
                view = xa_ref.at[b, pl.ds(base, n // 2), :]
                return jnp.concatenate([_upk16(view[r // 2:r // 2 + 8, :]) for r in range(0, n, 16)], axis=0)

            lhs_cache = {}

            def xa7():
                if 'a' not in lhs_cache:
                    lhs_cache['a'] = _lhs_f32(*_split4(xa_rows(r0, TQ)))
                return lhs_cache['a']

            def xe7():
                return _lhs_f32(*_split4(xa_rows(pl.multiple_of(t0, 16), TQ + 2 * PAD)))

            qparts = {}

            def q_piece(r):
                for k, v in enumerate(_lhs_combos(*oc(qm, r))):
                    q7[k, r // 2:(r + RB) // 2, :] = _pk(v)
                return []

            def u_piece(r):
                c11, c12, c21, c22 = [_gelu(v) for v in oc(um, r)]
                for half, pair in enumerate(((c11, c12), (c21, c22))):
                    for cb, blk in enumerate(pair):
                        for k in range(HD // 128):
                            u_ref[cb * (HD // 128) + k, half * H + r:half * H + r + RB, :] = (
                                blk[:, k * 128:(k + 1) * 128])
                return [(c11 + c12) + (c21 + c22)]

            def gt_piece(r, half, z=None):
                blocks = oc(gm, r)
                pre = jnp.concatenate(blocks[2 * half:2 * half + 2], axis=1)
                if z is not None:
                    pre = pre + jnp.concatenate([jnp.concatenate([z, z], axis=0)] * NC, axis=1)
                g = _ln(_gelu(pre))
                trow = lax.broadcasted_iota(jnp.int32, (RB, 128), 0) + (t0 - PAD + half * HE + r)
                valid = (trow >= 0) & (trow < T)
                outs = []
                for c in range(NC):
                    v = jnp.where(valid, g[:, c * 128:(c + 1) * 128], 0.0)
                    g_ref[c, half * HE + r:half * HE + r + RB, :] = v
                return []

            def kop(k, sl):
                return _upk(kc_ref[k, sl.start // 2:sl.stop // 2, :])

            km = [[None] * 7 for _ in range(NCH)]

            KORD = [1, 3, 2, 4, 0, 5, 6]

            def k_units(c):
                sl = slice(c * W, (c + 1) * W)

                def unit(k, toks):
                    km[c][k] = _dot_nt(tied(_upk(q7[k]), toks), kop(k, sl))
                    return km[c][k]
                return [functools.partial(unit, k) for k in KORD]

            stat = {}

            def k_piece(c, blk, r):
                sl = slice(c * W, (c + 1) * W)
                m = [None if v is None else v[r:r + RB, :] for v in km[c]]
                if blk == 0:
                    v = m[0] + m[3] - m[4] + m[6]
                elif blk == 1:
                    v = m[2] + m[4]
                elif blk == 2:
                    v = m[1] + m[3]
                else:
                    v = m[0] - m[1] + m[2] + m[5]
                if blk in (1, 3) and SH + (c + 1) * W > T:
                    col = lax.broadcasted_iota(jnp.int32, (RB, W), 1)
                    v = jnp.where(col < (T - SH - c * W), v, NEG)
                s_ref[blk + zs, r:r + RB, sl] = v
                tiles = [v[:, k * 128:(k + 1) * 128] for k in range(W // 128)]
                cm = functools.reduce(jnp.maximum, tiles)
                prev = stat.get((blk // 2, r))
                if prev is not None:
                    cm = jnp.maximum(cm, prev[0])
                l = functools.reduce(jnp.add, [jnp.exp2(t - cm) for t in tiles])
                if prev is not None:
                    l = l + prev[1] * jnp.exp2(prev[0] - cm)
                stat[blk // 2, r] = (cm, l)
                return [l]

            def k_pieces(c, blk):
                return [functools.partial(k_piece, c, blk, r) for r in ROWS]

            def fin(h):
                ms = jnp.concatenate([stat[h, r][0] for r in ROWS], axis=0)
                ls = jnp.concatenate([stat[h, r][1] for r in ROWS], axis=0)
                m = jnp.max(ms, axis=1, keepdims=True)
                return m + jnp.log2(jnp.sum(ls * jnp.exp2(ms - m), axis=1, keepdims=True))

            lb = jnp.where((s >= 1) & (s < NT), 1, 0)
            db = jnp.where(s < NT, 1, 0)
            lc = jnp.where(s < NT, jnp.maximum(s - 1, 0), (s - NT) % NLC)
            ln_pieces = [functools.partial(ln_rows, kn_ref, lb, db, lc, r) for r in range(0, LC, RB)]

            n = [None] * 7
            tmap = [0, 6, 1, 4, 5, 3, 2]
            off = []

            def fin_piece():
                off.extend([fin(0), fin(1)])
                return [jnp.broadcast_to(o, (H, 128)) for o in off]

            def p_units(c):
                sl = slice(c * W, (c + 1) * W)
                cache = {}

                def lhs(k):
                    if not cache:
                        cache['p'] = [jnp.exp2(s_ref[idx + zs, :, sl] - off[idx // 2]) for idx in range(4)]
                    p11, p12, p21, p22 = cache['p']
                    return [lambda: p11 + p22, lambda: p11, lambda: p21 - p22, lambda: p12 - p11,
                            lambda: p22, lambda: p11 + p21, lambda: p12 + p22][k]()

                def unit(k, toks):
                    r = _dot(tied_f32(lhs(k), toks).astype(BF16), kop(tmap[k], sl))
                    n[k] = r if n[k] is None else n[k] + r
                    return r
                return [functools.partial(unit, k) for k in (1, 4, 0, 3, 2, 5, 6)]

            zparts = {}

            def z_piece(c, r):
                vals = []
                for cc in (c, c + NC // 2):
                    for half in range(2):
                        rr = half * H + r
                        gc = conv_eo(g_ref, cwc_ref, cc, rr)
                        vals.append([u_ref[cc, pl.ds(rr + par, 8, stride=2), :] * gc[par] for par in range(2)])
                a11, a21, a12, a22 = vals
                store_lhs_eo(z7, r, c, a11, a12, a21, a22)
                return [a11[0] + a22[0], a11[1] + a22[1], a12[0] + a21[0], a12[1] + a21[1]]
            z_pieces = [functools.partial(z_piece, c, r) for r in ROWS for c in range(NC // 2)]
            lm = [None] * 7
            zc = {}

            def l_unit(k, toks):
                lm[k] = _dot(tied(_upk(z7[k]), toks), _upk(wout7[k]))
                return lm[k]

            def y_piece(r):
                n1, n2, n3, n4, n5, n6, n7 = [v[r:r + RB, :] for v in n]
                yb_ref[0, r:r + RB, :] = n1 + n4 - n5 + n7
                yb_ref[1, r:r + RB, :] = n2 + n4
                yb_ref[2, r:r + RB, :] = n3 + n5
                yb_ref[3, r:r + RB, :] = n1 - n2 + n3 + n6
                return []

            mc_pieces, mg_units, mg_pieces = merge_work()
            units = (g_units + mm_units(xa7, a7, qm) + mm_units(xa7, wu7, um) + mm_units(xe7, wg7, gm)
                     + k_units(0) + k_units(1) + k_units(2) + k_units(3) + mg_units
                     + p_units(0) + p_units(1) + p_units(2) + p_units(3)
                     + [functools.partial(l_unit, k) for k in range(7)])
            G, Q, U, TT, K0, K1, K2, K3, MG, P0, L = 0, 7, 14, 21, 28, 35, 42, 49, 56, 63, 91
            plan = {}
            spread(plan, g_pieces, Q + 2, U + 1)
            spread(plan, [functools.partial(q_piece, r) for r in ROWS], U + 2, TT + 1)
            spread(plan, [functools.partial(u_piece, r) for r in ROWS], TT + 2, K0 + 2)
            spread(plan, [functools.partial(gt_piece, r, h) for h in range(2) for r in ROWS_E],
                   K0 + 2, K0 + 13, lag=3)
            spread(plan, mc_pieces, K0 + 2, MG, lag=3)
            for c in range(NCH):
                u0 = K0 + 7 * c
                spread(plan, k_pieces(c, 2), u0 + 3, u0 + 4)
                spread(plan, k_pieces(c, 1), u0 + 5, u0 + 6)
                spread(plan, k_pieces(c, 3), u0 + 8, u0 + 9)
                spread(plan, k_pieces(c, 0), u0 + 9, u0 + 10)
            plan.setdefault(MG + 5, []).append((fin_piece, None))
            spread(plan, mg_pieces, P0 + 2, P0 + 8)
            for j, p in enumerate(ln_pieces):
                plan.setdefault(L, []).append((p, P0 + (j * 24) // len(ln_pieces)))
            spread(plan, z_pieces, P0 + 7, P0 + 27)
            spread(plan, [functools.partial(y_piece, r) for r in ROWS], L + 2, L + 6)
            run(units, plan)
            for p in store_m_pieces(NC, s, lm):
                p()

        @pl.when(s >= 3)
        def _():
            for_out(s - 2, lambda cp: cp.wait())

        @pl.when(s < NTT)
        def _():
            main_step()

        @pl.when(s >= NTT)
        def _():
            g_units, g_pieces = glob_work()
            run(g_units, {})
            for p in g_pieces:
                p()
            mc_pieces, mg_units, mg_pieces = merge_work()
            for p in mc_pieces:
                p()
            run(mg_units, {})
            for p in mg_pieces:
                p()

        @pl.when(s >= 1)
        def _():
            for_out(s, lambda cp: cp.start())

        @pl.when(s == NSTEPS - 1)
        def _():
            for_out(s - 1, lambda cp: cp.wait())
            for_out(s, lambda cp: cp.wait())

    anyspec = pl.BlockSpec(memory_space=pl.ANY)

    def full(shape):
        return pl.BlockSpec(shape, lambda s: (0,) * len(shape))

    return pl.pallas_call(
        kernel,
        grid=(NSTEPS,),
        in_specs=[anyspec, anyspec, anyspec, anyspec, full(dw_csgu.shape), anyspec,
                  full(dw_merge.shape), anyspec],
        out_specs=anyspec,
        out_shape=jax.ShapeDtypeStruct((B, T, D), x.dtype),
        scratch_shapes=[
            pltpu.VMEM((2, TQ, D), x.dtype),
            pltpu.VMEM((B, PAD + S, D), BF16),
            pltpu.VMEM((D, 3 * D), BF16),
            pltpu.VMEM((D, D), BF16),
            pltpu.VMEM((D, 2 * D), BF16),
            pltpu.VMEM((D, D), BF16),
            pltpu.VMEM((2 * D, D), BF16),
            pltpu.VMEM((B, XR // 2, D), U32),
            pltpu.VMEM((7, SH // 2, HD), U32),
            pltpu.VMEM((7, SH // 2, HD), U32),
            pltpu.VMEM((7, HD // 2, HD), U32),
            pltpu.VMEM((7, HD // 2, HD), U32),
            pltpu.VMEM((7, HD // 2, HD), U32),
            pltpu.VMEM((7, HD // 2, HD), U32),
            pltpu.VMEM((7, HD // 2, HD), U32),
            pltpu.VMEM((7, D // 2, HD), U32),
            pltpu.VMEM((KW, 8, D), F32),
            pltpu.VMEM((KW, 8, 2 * D), F32),
            pltpu.VMEM((4, H, SH), F32),
            pltpu.VMEM((4, H, HD), F32),
            pltpu.VMEM((7, H // 2, HD), U32),
            pltpu.VMEM((7, H // 2, HD), U32),
            pltpu.VMEM((7, H // 2, D), U32),
            pltpu.VMEM((NC, TQ, 128), F32),
            pltpu.VMEM((NC, TQ + 2 * PAD, 128), F32),
            pltpu.VMEM((2 * NC, MR, 128), F32),
            pltpu.SemaphoreType.DMA((6,)),
            pltpu.SemaphoreType.DMA((2 * NLC,)),
            pltpu.SemaphoreType.DMA((2,)),
        ],
        compiler_params=pltpu.CompilerParams(
            dimension_semantics=("arbitrary",), vmem_limit_bytes=110 * 1024 * 1024),
    )(x, w_qkv, w_att_out, w_mlp_in, dw_csgu, w_mlp_out, dw_merge, w_merge)
```

```python
import functools
import jax
import jax.numpy as jnp
from jax import lax
import jax.experimental.pallas as pl
import jax.experimental.pallas.tpu as pltpu

F32 = jnp.float32
BF16 = jnp.bfloat16
U32 = jnp.uint32
LOG2E = 1.4426950408889634
NT_DIMS = (((1,), (1,)), ((), ()))
NEG = -1e30


def _ln(xf, eps=1e-5):
    mu = jnp.mean(xf, axis=-1, keepdims=True)
    xc = xf - mu
    var = jnp.mean(xc * xc, axis=-1, keepdims=True)
    return xc * lax.rsqrt(var + eps)


def _gelu(x):
    c0 = 0.7978845608028654
    c1 = 0.7978845608028654 * 0.044715
    inner = x * (c0 + c1 * (x * x))
    hx = 0.5 * x
    return hx + hx * jnp.tanh(inner)


def _dot(a, b):
    return jnp.dot(a, b, preferred_element_type=F32)


def _dot_nt(a, b):
    return lax.dot_general(a, b, NT_DIMS, preferred_element_type=F32)


def _lhs_f32(a11, a12, a21, a22):
    return [a11 + a22, a21 + a22, a11, a22, a11 + a12, a21 - a11, a12 - a22]


def _lhs_combos(a11, a12, a21, a22):
    return [v.astype(BF16) for v in _lhs_f32(a11, a12, a21, a22)]


def _rhs_combos(b11, b12, b21, b22):
    return [b11 + b22, b11, b12 - b22, b21 - b11, b22, b11 + b12, b21 + b22]


def _out_combos(m1, m2, m3, m4, m5, m6, m7):
    return m1 + m4 - m5 + m7, m3 + m5, m2 + m4, m1 - m2 + m3 + m6


def _split4(a):
    r, c = a.shape
    h, w = r // 2, c // 2
    return a[:h, :w], a[:h, w:], a[h:, :w], a[h:, w:]


def _pk(v):
    return pltpu.bitcast(v, U32)


def _upk(v):
    return pltpu.bitcast(v, BF16)


def _pk16(v):
    return _pk(v.astype(BF16))


def _upk16(w):
    return _upk(w).astype(F32)


def _token(vals):
    tiles = []
    for v in vals:
        b = pltpu.bitcast(v, U32)
        r, c = b.shape
        tiles += [b[i:i + 8, j:j + 128] for i in range(0, r, 8) for j in range(0, c, 128)]
    return functools.reduce(jnp.bitwise_or, tiles)


def _cat7(parts, rows, cols):
    return [jnp.concatenate(
        [jnp.concatenate([parts[r, c][k] for c in cols], axis=1) if len(cols) > 1 else parts[r, cols[0]][k]
         for r in rows], axis=0) for k in range(7)]


@jax.jit
def pallas_standalone__conformer_family_e_branchformer__speech_kernel(
    x, w_qkv, w_att_out, w_mlp_in, dw_csgu, w_mlp_out, dw_merge, w_merge):
    B, T, D = x.shape
    KW = dw_csgu.shape[0]
    assert KW == 5 and B == 2
    TQ = 448
    H = TQ // 2
    HD = D // 2
    NT = pl.cdiv(T, TQ)
    PAD = 16
    HE = (TQ + 2 * PAD) // 2
    S = 4096
    SH = S // 2
    W = 512
    NCH = SH // W
    LC = 256
    NLC = SH // LC
    XR = PAD + S + PAD
    MH = 2 * PAD
    MR = MH + TQ
    NC = D // 128
    NTT = B * NT
    NSTEPS = NTT + 1
    scale = float(D) ** -0.5 * LOG2E
    RB = 16
    ROWS = list(range(0, H, RB))
    ROWS_E = list(range(0, HE, RB))

    def kernel(x_hbm, wqkv_hbm, wo_hbm, win_hbm, dwc_ref, wout_hbm, dwm_ref, wm_hbm,
               o_hbm,
               ob_ref, x_ref, wqkv_ref, wo_ref, win_ref, wout_ref, wm_ref,
               xa_ref, kc_ref, kn_ref, a7, wu7, wg7, wout7, wvo7, wm7,
               cwc_ref, cwm_ref,
               s_ref, yb_ref, q7, z7, ml7, u_ref, g_ref, m_ref,
               sems, xsems, osems):
        s = pl.program_id(0)
        zs = s >> 30
        zero = jnp.full((8, 128), zs, jnp.int32).astype(U32)

        def ln_rows(kdst, sb, db, c, r, z=None):
            rl = pl.multiple_of(c * LC + r, 16)
            rr = pl.multiple_of(SH + c * LC + r, 16)
            xl = x_ref[sb, pl.ds(PAD + rl, RB), :].astype(F32)
            xr = x_ref[sb, pl.ds(PAD + rr, RB), :].astype(F32)
            if z is not None:
                z2 = jnp.concatenate([z, z], axis=0)
                xl = jnp.concatenate([xl[:, :128] + z2, xl[:, 128:]], axis=1)
                xr = jnp.concatenate([xr[:, :128] + z2, xr[:, 128:]], axis=1)
            xl = _ln(xl)
            xr = _ln(xr)
            l1, l2, r1, r2 = xl[:, :HD], xl[:, HD:], xr[:, :HD], xr[:, HD:]
            hl = pl.multiple_of((c * LC + r) // 2, 8)
            xa_ref[db, pl.ds(PAD // 2 + hl, 8), :] = _pk16(xl)
            xa_ref[db, pl.ds((PAD + SH) // 2 + hl, 8), :] = _pk16(xr)
            for k, v in enumerate([l1 + r2, l1, r1 - r2, l2 - l1, r2, l1 + r1, l2 + r2]):
                kdst[k, pl.ds(hl, 8), :] = _pk16(v)
            return [l1 + r1, l2 + r2]

        def w_copy(i):
            srcs = [(wqkv_hbm, wqkv_ref), (wo_hbm, wo_ref), (win_hbm, win_ref), (wout_hbm, wout_ref),
                    (wm_hbm, wm_ref)]
            return pltpu.make_async_copy(srcs[i][0], srcs[i][1], sems.at[i])

        def x0_copy(c, h, n=LC):
            r = h * SH + c * LC
            if not isinstance(r, int):
                r = pl.multiple_of(r, LC)
            return pltpu.make_async_copy(x_hbm.at[0, pl.ds(r, n), :], x_ref.at[0, pl.ds(PAD + r, n), :],
                                         xsems.at[2 * c + h])

        def x1_copy():
            return pltpu.make_async_copy(x_hbm.at[1], x_ref.at[1, pl.ds(PAD, T), :], sems.at[5])

        def set_w7(dst, w):
            for k, v in enumerate(_rhs_combos(*_split4(w))):
                dst[k] = _pk(v.astype(BF16))

        @pl.when(s == 0)
        def _prologue():
            NLAST = T - SH - (NLC - 1) * LC
            for c in range(NLC):
                x0_copy(c, 0).start()
                x0_copy(c, 1, LC if c < NLC - 1 else NLAST).start()
            w_copy(0).start()
            w_copy(1).start()
            w_copy(2).start()
            w_copy(3).start()
            for b in range(B):
                x_ref[b, 0:PAD, :] = jnp.zeros((PAD, D), BF16)
                x_ref[b, PAD + T:PAD + S, :] = jnp.zeros((S - T, D), BF16)
                xa_ref[b, 0:PAD // 2, :] = jnp.zeros((PAD // 2, D), U32)
                xa_ref[b, (PAD + S) // 2:XR // 2, :] = jnp.zeros((PAD // 2, D), U32)
            m_ref[...] = jnp.zeros(m_ref.shape, F32)
            for d in range(KW):
                cwc_ref[d] = jnp.broadcast_to(dwc_ref[d:d + 1, :].astype(F32), (8, D))
                w = dwm_ref[d:d + 1, :].astype(F32)
                if d == KW // 2:
                    w = w + 1.0
                cwm_ref[d] = jnp.broadcast_to(w, (8, 2 * D))
            yb_ref[...] = jnp.zeros(yb_ref.shape, F32)
            def ln_chunk0(c):
                for r in range(0, LC, RB):
                    ln_rows(kc_ref, 0, 0, c, r)

            def body(c, carry):
                x0_copy(c, 0).wait()
                x0_copy(c, 1).wait()
                ln_chunk0(c)
                return carry
            lax.fori_loop(0, NLC - 1, body, 0)
            x0_copy(NLC - 1, 0).wait()
            x0_copy(NLC - 1, 1, NLAST).wait()
            lax.fori_loop(NLC - 1, NLC, lambda c, carry: (ln_chunk0(c), carry)[1], 0)
            w_copy(0).wait()
            set_w7(a7, _dot_nt(wqkv_ref[:, 0:D], wqkv_ref[:, D:2 * D]) * scale)
            w_copy(1).wait()
            set_w7(wvo7, _dot(wqkv_ref[:, 2 * D:3 * D], wo_ref[...]))
            w_copy(4).start()
            x1_copy().start()
            w_copy(2).wait()
            set_w7(wu7, win_ref[:, 0:D].astype(F32))
            set_w7(wg7, win_ref[:, D:2 * D].astype(F32))
            w_copy(3).wait()
            set_w7(wout7, wout_ref[...].astype(F32))
            wm7[...] = jnp.zeros(wm7.shape, U32)

        @pl.when(s == 1)
        def _():
            x1_copy().wait()
            w_copy(4).wait()
            set_w7(wm7, wm_ref[...].astype(F32))

        @pl.when(s == NT)
        def _():
            def body(j, carry):
                r = pl.multiple_of(j * 64, 64)
                for k in range(7):
                    kc_ref[k, pl.ds(r, 64), :] = kn_ref[k, pl.ds(r, 64), :]
                return carry
            lax.fori_loop(0, SH // 2 // 64, body, 0)

        def tie_head(head_u32, toks):
            return head_u32 | (functools.reduce(jnp.bitwise_or, toks) & zero)

        def zero_after(v):
            return pltpu.bitcast(pltpu.bitcast(v[:8, :128], U32) & zero, F32)

        def tied(lhs, toks):
            if not toks:
                return lhs
            head = _upk(tie_head(_pk(lhs[:16, :128]), toks))
            return jnp.concatenate(
                [jnp.concatenate([head, lhs[:16, 128:]], axis=1), lhs[16:]], axis=0)

        def tied_f32(lhs, toks):
            if not toks:
                return lhs
            head = pltpu.bitcast(tie_head(pltpu.bitcast(lhs[:8, :128], U32), toks), F32)
            return jnp.concatenate(
                [jnp.concatenate([head, lhs[:8, 128:]], axis=1), lhs[8:]], axis=0)

        def mm_units(get_lhs7, w_ref, out):
            cache = {}

            def unit(k, toks):
                if not cache:
                    cache['l'] = get_lhs7()
                out[k] = _dot(tied_f32(cache['l'][k], toks).astype(BF16), _upk(w_ref[k]))
                return out[k]
            return [functools.partial(unit, k) for k in range(7)]

        def oc(ms, r, n=RB):
            return _out_combos(*[m[r:r + n, :] for m in ms])

        def store_m_pieces(c0, tile, ms):
            t0 = (tile % NT) * TQ

            def tail():
                keep = (tile % NT) > 0
                for c in range(c0, c0 + NC):
                    m_ref[c, 0:MH, :] = jnp.where(keep, m_ref[c, TQ:TQ + MH, :], 0.0)
                return []

            def piece(r):
                blocks = oc(ms, r)
                row = lax.broadcasted_iota(jnp.int32, (RB, 128), 0)
                for half in range(2):
                    valid = (row + (t0 + half * H + r)) < T
                    for cb in range(2):
                        blk = blocks[2 * half + cb]
                        for k in range(HD // 128):
                            rr = MH + half * H + r
                            m_ref[c0 + cb * (HD // 128) + k, rr:rr + RB, :] = (
                                jnp.where(valid, blk[:, k * 128:(k + 1) * 128], 0.0))
                return []
            return [tail] + [functools.partial(piece, r) for r in ROWS]

        def conv_block(ref, cw_ref, c, r, n, z=None):
            acc = None
            for d in range(KW):
                w = cw_ref[d, :, c * 128:(c + 1) * 128]
                if z is not None:
                    w = w + z
                w = jnp.concatenate([w] * (n // 8), axis=0)
                v = ref[c, PAD - 2 + d + r:PAD - 2 + d + r + n, :] * w
                acc = v if acc is None else acc + v
            return acc

        def glob_work():
            ms = [None] * 7
            units = mm_units(lambda: _lhs_f32(*[yb_ref[q] for q in range(4)]), wvo7, ms)
            return units, store_m_pieces(0, jnp.maximum(s - 1, 0), ms)

        def merge_work():
            jg = jnp.maximum(s - 1, 0)
            b = jg // NT
            base = pl.multiple_of((jg % NT) * TQ, 16)
            slot = s % 2

            def lhs_piece(c, r, z=None):
                a11 = conv_block(m_ref, cwm_ref, c, r, RB, z)
                a21 = conv_block(m_ref, cwm_ref, c, H + r, RB, z)
                a12 = conv_block(m_ref, cwm_ref, NC + c, r, RB, z)
                a22 = conv_block(m_ref, cwm_ref, NC + c, H + r, RB, z)
                for k, v in enumerate(_lhs_combos(a11, a12, a21, a22)):
                    ml7[k, r // 2:(r + RB) // 2, c * 128:(c + 1) * 128] = _pk(v)
                return []
            lhs_pieces = [functools.partial(lhs_piece, c, r) for r in ROWS for c in range(NC)]
            ms = [None] * 7

            def unit(k, toks):
                ms[k] = _dot(tied(_upk(ml7[k]), toks), _upk(wm7[k]))
                return ms[k]

            def piece(r):
                c11, c12, c21, c22 = oc(ms, r)
                for half, (lo, hi) in enumerate(((c11, c12), (c21, c22))):
                    xr = x_ref[b, pl.ds(pl.multiple_of(base + half * H + r, 16), RB), :].astype(F32)
                    ob_ref[slot, half * H + r:half * H + r + RB, :] = (
                        xr + jnp.concatenate([lo, hi], axis=1)).astype(ob_ref.dtype)
                return []
            return (lhs_pieces, [functools.partial(unit, k) for k in range(7)],
                    [functools.partial(piece, r) for r in ROWS])

        def out_copy(step, kind):
            jg = step - 1
            b = jg // NT
            j = jg % NT
            slot = step % 2
            if kind == 0:
                src_, off, n = ob_ref.at[slot, pl.ds(PAD, TQ - PAD), :], 0, TQ - PAD
            elif kind == 1:
                src_, off, n = ob_ref.at[slot], pl.multiple_of(j * TQ - PAD, 16), TQ
            else:
                n = T - ((NT - 1) * TQ - PAD)
                src_, off = ob_ref.at[slot, pl.ds(0, n), :], (NT - 1) * TQ - PAD
            return pltpu.make_async_copy(src_, o_hbm.at[b, pl.ds(off, n), :], osems.at[slot])

        def for_out(step, fn):
            j = (step - 1) % NT
            for kind, cond in enumerate((j == 0, (j > 0) & (j < NT - 1), j == NT - 1)):
                @pl.when(cond)
                def _(kind=kind):
                    fn(out_copy(step, kind))

        def run(units, plan):
            outs = []
            for i, u in enumerate(units):
                toks = []
                for p, a in plan.get(i, []):
                    vals = p() if a is None else p(z=zero_after(outs[a]))
                    if vals:
                        toks.append(_token(vals))
                outs.append(u(toks))

        def spread(plan, pieces, lo, hi, lag=None):
            n = hi - lo + 1
            for j, p in enumerate(pieces):
                i = lo + (j * n) // len(pieces)
                plan.setdefault(i, []).append((p, None if lag is None else i - lag))

        def main_step():
            b = s // NT
            i = s % NT
            t0 = i * TQ
            r0 = pl.multiple_of(PAD + t0, 16)

            g_units, g_pieces = glob_work()
            qm, um, gm = [None] * 7, [None] * 7, [None] * 7

            def xa_rows(row0, n):
                base = pl.multiple_of(row0 // 2, 8)
                view = xa_ref.at[b, pl.ds(base, n // 2), :]
                return jnp.concatenate([_upk16(view[r // 2:r // 2 + 8, :]) for r in range(0, n, 16)], axis=0)

            lhs_cache = {}

            def xa7():
                if 'a' not in lhs_cache:
                    lhs_cache['a'] = _lhs_f32(*_split4(xa_rows(r0, TQ)))
                return lhs_cache['a']

            def xe7():
                return _lhs_f32(*_split4(xa_rows(pl.multiple_of(t0, 16), TQ + 2 * PAD)))

            qparts = {}

            def q_piece(r):
                for k, v in enumerate(_lhs_combos(*oc(qm, r))):
                    q7[k, r // 2:(r + RB) // 2, :] = _pk(v)
                return []

            def u_piece(r):
                c11, c12, c21, c22 = [_gelu(v) for v in oc(um, r)]
                u_ref[r:r + RB, 0:HD] = c11
                u_ref[r:r + RB, HD:D] = c12
                u_ref[H + r:H + r + RB, 0:HD] = c21
                u_ref[H + r:H + r + RB, HD:D] = c22
                return [(c11 + c12) + (c21 + c22)]

            def gt_piece(r, half, z=None):
                blocks = oc(gm, r)
                pre = jnp.concatenate(blocks[2 * half:2 * half + 2], axis=1)
                if z is not None:
                    pre = pre + jnp.concatenate([jnp.concatenate([z, z], axis=0)] * NC, axis=1)
                g = _ln(_gelu(pre))
                trow = lax.broadcasted_iota(jnp.int32, (RB, 128), 0) + (t0 - PAD + half * HE + r)
                valid = (trow >= 0) & (trow < T)
                outs = []
                for c in range(NC):
                    v = jnp.where(valid, g[:, c * 128:(c + 1) * 128], 0.0)
                    g_ref[c, half * HE + r:half * HE + r + RB, :] = v
                return []

            def kop(k, sl):
                return _upk(kc_ref[k, sl.start // 2:sl.stop // 2, :])

            km = [[None] * 7 for _ in range(NCH)]

            KORD = [1, 3, 2, 4, 0, 5, 6]

            def k_units(c):
                sl = slice(c * W, (c + 1) * W)

                def unit(k, toks):
                    km[c][k] = _dot_nt(tied(_upk(q7[k]), toks), kop(k, sl))
                    return km[c][k]
                return [functools.partial(unit, k) for k in KORD]

            stat = {}

            def k_piece(c, blk, r):
                sl = slice(c * W, (c + 1) * W)
                m = [None if v is None else v[r:r + RB, :] for v in km[c]]
                if blk == 0:
                    v = m[0] + m[3] - m[4] + m[6]
                elif blk == 1:
                    v = m[2] + m[4]
                elif blk == 2:
                    v = m[1] + m[3]
                else:
                    v = m[0] - m[1] + m[2] + m[5]
                if blk in (1, 3) and SH + (c + 1) * W > T:
                    col = lax.broadcasted_iota(jnp.int32, (RB, W), 1)
                    v = jnp.where(col < (T - SH - c * W), v, NEG)
                s_ref[blk + zs, r:r + RB, sl] = v
                tiles = [v[:, k * 128:(k + 1) * 128] for k in range(W // 128)]
                cm = functools.reduce(jnp.maximum, tiles)
                prev = stat.get((blk // 2, r))
                if prev is not None:
                    cm = jnp.maximum(cm, prev[0])
                l = functools.reduce(jnp.add, [jnp.exp2(t - cm) for t in tiles])
                if prev is not None:
                    l = l + prev[1] * jnp.exp2(prev[0] - cm)
                stat[blk // 2, r] = (cm, l)
                return [l]

            def k_pieces(c, blk):
                return [functools.partial(k_piece, c, blk, r) for r in ROWS]

            def fin(h):
                ms = jnp.concatenate([stat[h, r][0] for r in ROWS], axis=0)
                ls = jnp.concatenate([stat[h, r][1] for r in ROWS], axis=0)
                m = jnp.max(ms, axis=1, keepdims=True)
                return m + jnp.log2(jnp.sum(ls * jnp.exp2(ms - m), axis=1, keepdims=True))

            lb = jnp.where((s >= 1) & (s < NT), 1, 0)
            db = jnp.where(s < NT, 1, 0)
            lc = jnp.where(s < NT, jnp.maximum(s - 1, 0), (s - NT) % NLC)
            ln_pieces = [functools.partial(ln_rows, kn_ref, lb, db, lc, r) for r in range(0, LC, RB)]

            n = [None] * 7
            tmap = [0, 6, 1, 4, 5, 3, 2]
            off = []

            def fin_piece():
                off.extend([fin(0), fin(1)])
                return [jnp.broadcast_to(o, (H, 128)) for o in off]

            def p_units(c):
                sl = slice(c * W, (c + 1) * W)
                cache = {}

                def lhs(k):
                    if not cache:
                        cache['p'] = [jnp.exp2(s_ref[idx + zs, :, sl] - off[idx // 2]) for idx in range(4)]
                    p11, p12, p21, p22 = cache['p']
                    return [lambda: p11 + p22, lambda: p11, lambda: p21 - p22, lambda: p12 - p11,
                            lambda: p22, lambda: p11 + p21, lambda: p12 + p22][k]()

                def unit(k, toks):
                    r = _dot(tied_f32(lhs(k), toks).astype(BF16), kop(tmap[k], sl))
                    n[k] = r if n[k] is None else n[k] + r
                    return r
                return [functools.partial(unit, k) for k in (1, 4, 0, 3, 2, 5, 6)]

            zparts = {}

            def z_piece(c, r):
                vals = []
                for cc in (c, c + NC // 2):
                    for half in range(2):
                        rr = half * H + r
                        gc = conv_block(g_ref, cwc_ref, cc, rr, RB)
                        vals.append(u_ref[rr:rr + RB, cc * 128:(cc + 1) * 128] * gc)
                a11, a21, a12, a22 = vals
                for k, v in enumerate(_lhs_combos(a11, a12, a21, a22)):
                    z7[k, r // 2:(r + RB) // 2, c * 128:(c + 1) * 128] = _pk(v)
                return [a11 + a22, a12 + a21]
            z_pieces = [functools.partial(z_piece, c, r) for r in ROWS for c in range(NC // 2)]
            lm = [None] * 7
            zc = {}

            def l_unit(k, toks):
                lm[k] = _dot(tied(_upk(z7[k]), toks), _upk(wout7[k]))
                return lm[k]

            def y_piece(r):
                n1, n2, n3, n4, n5, n6, n7 = [v[r:r + RB, :] for v in n]
                yb_ref[0, r:r + RB, :] = n1 + n4 - n5 + n7
                yb_ref[1, r:r + RB, :] = n2 + n4
                yb_ref[2, r:r + RB, :] = n3 + n5
                yb_ref[3, r:r + RB, :] = n1 - n2 + n3 + n6
                return []

            mc_pieces, mg_units, mg_pieces = merge_work()
            units = (g_units + mm_units(xa7, a7, qm) + mm_units(xa7, wu7, um) + mm_units(xe7, wg7, gm)
                     + k_units(0) + k_units(1) + k_units(2) + k_units(3) + mg_units
                     + p_units(0) + p_units(1) + p_units(2) + p_units(3)
                     + [functools.partial(l_unit, k) for k in range(7)])
            G, Q, U, TT, K0, K1, K2, K3, MG, P0, L = 0, 7, 14, 21, 28, 35, 42, 49, 56, 63, 91
            plan = {}
            spread(plan, g_pieces, Q + 2, U + 1)
            spread(plan, [functools.partial(q_piece, r) for r in ROWS], U + 2, TT + 1)
            spread(plan, [functools.partial(u_piece, r) for r in ROWS], TT + 2, K0 + 2)
            spread(plan, [functools.partial(gt_piece, r, h) for h in range(2) for r in ROWS_E],
                   K0 + 2, K0 + 13, lag=3)
            spread(plan, mc_pieces, K0 + 2, MG, lag=3)
            for c in range(NCH):
                u0 = K0 + 7 * c
                spread(plan, k_pieces(c, 2), u0 + 3, u0 + 4)
                spread(plan, k_pieces(c, 1), u0 + 5, u0 + 6)
                spread(plan, k_pieces(c, 3), u0 + 8, u0 + 9)
                spread(plan, k_pieces(c, 0), u0 + 9, u0 + 10)
            plan.setdefault(MG + 4, []).append((fin_piece, None))
            spread(plan, mg_pieces, P0 + 2, P0 + 8)
            for j, p in enumerate(ln_pieces):
                plan.setdefault(L, []).append((p, P0 + (j * 24) // len(ln_pieces)))
            spread(plan, z_pieces, P0 + 7, P0 + 27)
            spread(plan, [functools.partial(y_piece, r) for r in ROWS], L + 2, L + 6)
            run(units, plan)
            for p in store_m_pieces(NC, s, lm):
                p()

        @pl.when(s >= 3)
        def _():
            for_out(s - 2, lambda cp: cp.wait())

        @pl.when(s < NTT)
        def _():
            main_step()

        @pl.when(s >= NTT)
        def _():
            g_units, g_pieces = glob_work()
            run(g_units, {})
            for p in g_pieces:
                p()
            mc_pieces, mg_units, mg_pieces = merge_work()
            for p in mc_pieces:
                p()
            run(mg_units, {})
            for p in mg_pieces:
                p()

        @pl.when(s >= 1)
        def _():
            for_out(s, lambda cp: cp.start())

        @pl.when(s == NSTEPS - 1)
        def _():
            for_out(s - 1, lambda cp: cp.wait())
            for_out(s, lambda cp: cp.wait())

    anyspec = pl.BlockSpec(memory_space=pl.ANY)

    def full(shape):
        return pl.BlockSpec(shape, lambda s: (0,) * len(shape))

    return pl.pallas_call(
        kernel,
        grid=(NSTEPS,),
        in_specs=[anyspec, anyspec, anyspec, anyspec, full(dw_csgu.shape), anyspec,
                  full(dw_merge.shape), anyspec],
        out_specs=anyspec,
        out_shape=jax.ShapeDtypeStruct((B, T, D), x.dtype),
        scratch_shapes=[
            pltpu.VMEM((2, TQ, D), x.dtype),
            pltpu.VMEM((B, PAD + S, D), BF16),
            pltpu.VMEM((D, 3 * D), BF16),
            pltpu.VMEM((D, D), BF16),
            pltpu.VMEM((D, 2 * D), BF16),
            pltpu.VMEM((D, D), BF16),
            pltpu.VMEM((2 * D, D), BF16),
            pltpu.VMEM((B, XR // 2, D), U32),
            pltpu.VMEM((7, SH // 2, HD), U32),
            pltpu.VMEM((7, SH // 2, HD), U32),
            pltpu.VMEM((7, HD // 2, HD), U32),
            pltpu.VMEM((7, HD // 2, HD), U32),
            pltpu.VMEM((7, HD // 2, HD), U32),
            pltpu.VMEM((7, HD // 2, HD), U32),
            pltpu.VMEM((7, HD // 2, HD), U32),
            pltpu.VMEM((7, D // 2, HD), U32),
            pltpu.VMEM((KW, 8, D), F32),
            pltpu.VMEM((KW, 8, 2 * D), F32),
            pltpu.VMEM((4, H, SH), F32),
            pltpu.VMEM((4, H, HD), F32),
            pltpu.VMEM((7, H // 2, HD), U32),
            pltpu.VMEM((7, H // 2, HD), U32),
            pltpu.VMEM((7, H // 2, D), U32),
            pltpu.VMEM((TQ, D), F32),
            pltpu.VMEM((NC, TQ + 2 * PAD, 128), F32),
            pltpu.VMEM((2 * NC, MR, 128), F32),
            pltpu.SemaphoreType.DMA((6,)),
            pltpu.SemaphoreType.DMA((2 * NLC,)),
            pltpu.SemaphoreType.DMA((2,)),
        ],
        compiler_params=pltpu.CompilerParams(
            dimension_semantics=("arbitrary",), vmem_limit_bytes=110 * 1024 * 1024),
    )(x, w_qkv, w_att_out, w_mlp_in, dw_csgu, w_mlp_out, dw_merge, w_merge)
```

```python
import functools
import jax
import jax.numpy as jnp
from jax import lax
import jax.experimental.pallas as pl
import jax.experimental.pallas.tpu as pltpu

F32 = jnp.float32
BF16 = jnp.bfloat16
U32 = jnp.uint32
LOG2E = 1.4426950408889634
NT_DIMS = (((1,), (1,)), ((), ()))
NEG = -1e30


def _ln(xf, eps=1e-5):
    mu = jnp.mean(xf, axis=-1, keepdims=True)
    xc = xf - mu
    var = jnp.mean(xc * xc, axis=-1, keepdims=True)
    return xc * lax.rsqrt(var + eps)


def _gelu(x):
    c0 = 0.7978845608028654
    c1 = 0.7978845608028654 * 0.044715
    inner = x * (c0 + c1 * (x * x))
    hx = 0.5 * x
    return hx + hx * jnp.tanh(inner)


def _dot(a, b):
    return jnp.dot(a, b, preferred_element_type=F32)


def _dot_nt(a, b):
    return lax.dot_general(a, b, NT_DIMS, preferred_element_type=F32)


def _lhs_f32(a11, a12, a21, a22):
    return [a11 + a22, a21 + a22, a11, a22, a11 + a12, a21 - a11, a12 - a22]


def _lhs_combos(a11, a12, a21, a22):
    return [v.astype(BF16) for v in _lhs_f32(a11, a12, a21, a22)]


def _rhs_combos(b11, b12, b21, b22):
    return [b11 + b22, b11, b12 - b22, b21 - b11, b22, b11 + b12, b21 + b22]


def _out_block(blk, m):
    if blk == 0:
        return m[0] + m[3] - m[4] + m[6]
    if blk == 1:
        return m[2] + m[4]
    if blk == 2:
        return m[1] + m[3]
    return m[0] - m[1] + m[2] + m[5]


def _out_combos(*m):
    return tuple(_out_block(blk, m) for blk in range(4))


def _split4(a):
    r, c = a.shape
    h, w = r // 2, c // 2
    return a[:h, :w], a[:h, w:], a[h:, :w], a[h:, w:]


def _pk(v):
    return pltpu.bitcast(v, U32)


def _upk(v):
    return pltpu.bitcast(v, BF16)


def _pk16(v):
    return _pk(v.astype(BF16))


def _upk16(w):
    return _upk(w).astype(F32)


def _token(vals):
    tiles = []
    for v in vals:
        b = pltpu.bitcast(v, U32)
        r, c = b.shape
        tiles += [b[i:i + 8, j:j + 128] for i in range(0, r, 8) for j in range(0, c, 128)]
    return functools.reduce(jnp.bitwise_or, tiles)


@jax.jit
def pallas_standalone__conformer_family_e_branchformer__speech_kernel(
    x, w_qkv, w_att_out, w_mlp_in, dw_csgu, w_mlp_out, dw_merge, w_merge):
    B, T, D = x.shape
    KW = dw_csgu.shape[0]
    assert KW == 5 and B == 2
    TQ = 448
    H = TQ // 2
    HD = D // 2
    NT = pl.cdiv(T, TQ)
    PAD = 16
    S = 4096
    SH = S // 2
    W = 512
    NCH = SH // W
    LC = 256
    NLC = SH // LC
    XR = PAD + S + PAD
    PX = 2 * PAD
    MG_H, ML_H = 3 * PAD, 2 * PAD
    MR = MG_H + TQ
    GH = 2 * PAD
    NC = D // 128
    NTT = B * NT
    NSTEPS = NTT + 1
    scale = float(D) ** -0.5 * LOG2E
    RB = 16
    ROWS = list(range(0, H, RB))

    def kernel(x_hbm, wqkv_hbm, wo_hbm, win_hbm, dwc_ref, wout_hbm, dwm_ref, wm_hbm,
               o_hbm,
               ob_ref, x_ref, wqkv_ref, wo_ref, win_ref, wout_ref, wm_ref,
               xa_ref, kc_ref, kn_ref, a7, win7, wout7, wvo7, wm7,
               cwc_ref, cwm_ref,
               s_ref, yb_ref, q7, z7, ml7, u_ref, g_ref, m_ref,
               sems, xsems, osems):
        s = pl.program_id(0)
        zs = s >> 30
        zero = jnp.full((8, 128), zs, jnp.int32).astype(U32)

        def ln_rows(kdst, sb, db, c, r, z=None):
            rl = pl.multiple_of(c * LC + r, 16)
            rr = pl.multiple_of(SH + c * LC + r, 16)
            xl = x_ref[sb, pl.ds(PX + rl, RB), :].astype(F32)
            xr = x_ref[sb, pl.ds(PX + rr, RB), :].astype(F32)
            if z is not None:
                z2 = jnp.concatenate([z, z], axis=0)
                xl = jnp.concatenate([xl[:, :128] + z2, xl[:, 128:]], axis=1)
                xr = jnp.concatenate([xr[:, :128] + z2, xr[:, 128:]], axis=1)
            xl = _ln(xl)
            xr = _ln(xr)
            l1, l2, r1, r2 = xl[:, :HD], xl[:, HD:], xr[:, :HD], xr[:, HD:]
            hl = pl.multiple_of((c * LC + r) // 2, 8)
            xa_ref[db, pl.ds(PAD // 2 + hl, 8), :] = _pk16(xl)
            xa_ref[db, pl.ds((PAD + SH) // 2 + hl, 8), :] = _pk16(xr)
            for k, v in enumerate([l1 + r2, l1, r1 - r2, l2 - l1, r2, l1 + r1, l2 + r2]):
                kdst[k, pl.ds(hl, 8), :] = _pk16(v)
            return [l1 + r1, l2 + r2]

        def w_copy(i):
            srcs = [(wqkv_hbm, wqkv_ref), (wo_hbm, wo_ref), (win_hbm, win_ref), (wout_hbm, wout_ref),
                    (wm_hbm, wm_ref)]
            return pltpu.make_async_copy(srcs[i][0], srcs[i][1], sems.at[i])

        def x0_copy(c, h, n=LC):
            r = h * SH + c * LC
            if not isinstance(r, int):
                r = pl.multiple_of(r, LC)
            return pltpu.make_async_copy(x_hbm.at[0, pl.ds(r, n), :], x_ref.at[0, pl.ds(PX + r, n), :],
                                         xsems.at[2 * c + h])

        def x1_copy():
            return pltpu.make_async_copy(x_hbm.at[1], x_ref.at[1, pl.ds(PX, T), :], sems.at[5])

        def set_w7(dst, w):
            for k, v in enumerate(_rhs_combos(*_split4(w))):
                dst[k] = _pk(v.astype(BF16))

        @pl.when(s == 0)
        def _prologue():
            NLAST = T - SH - (NLC - 1) * LC
            NLOOP = NLC - 4

            def x0_pair(c):
                return [x0_copy(c, 0), x0_copy(c, 1, LC if c < NLC - 1 else NLAST)]
            order = ([x0_pair(c) for c in range(NLOOP)] + [[w_copy(0)], x0_pair(NLOOP), x0_pair(NLOOP + 1),
                     [w_copy(1)], x0_pair(NLOOP + 2), x0_pair(NLOOP + 3), [w_copy(2)], [w_copy(3)]])
            for group in order:
                for cp in group:
                    cp.start()
            for b in range(B):
                x_ref[b, 0:PX, :] = jnp.zeros((PX, D), BF16)
                x_ref[b, PX + T:PX + S, :] = jnp.zeros((S - T, D), BF16)
                xa_ref[b, 0:PAD // 2, :] = jnp.zeros((PAD // 2, D), U32)
                xa_ref[b, (PAD + S) // 2:XR // 2, :] = jnp.zeros((PAD // 2, D), U32)
            m_ref[...] = jnp.zeros(m_ref.shape, F32)
            u_ref[...] = jnp.zeros(u_ref.shape, F32)
            g_ref[...] = jnp.zeros(g_ref.shape, F32)
            for d in range(KW):
                cwc_ref[d] = jnp.broadcast_to(dwc_ref[d:d + 1, :].astype(F32), (8, D))
                w = dwm_ref[d:d + 1, :].astype(F32)
                if d == KW // 2:
                    w = w + 1.0
                cwm_ref[d] = jnp.broadcast_to(w, (8, 2 * D))
            yb_ref[...] = jnp.zeros(yb_ref.shape, F32)

            def ln_chunk0(c):
                for r in range(0, LC, RB):
                    ln_rows(kc_ref, 0, 0, c, r)

            def body(c, carry):
                x0_copy(c, 0).wait()
                x0_copy(c, 1).wait()
                ln_chunk0(c)
                return carry
            lax.fori_loop(0, NLOOP, body, 0)
            for cp in [w_copy(0)] + x0_pair(NLOOP) + x0_pair(NLOOP + 1):
                cp.wait()
            set_w7(a7, _dot_nt(wqkv_ref[:, 0:D], wqkv_ref[:, D:2 * D]) * scale)
            ln_chunk0(NLOOP)
            ln_chunk0(NLOOP + 1)
            for cp in [w_copy(1)] + x0_pair(NLOOP + 2) + x0_pair(NLOOP + 3):
                cp.wait()
            set_w7(wvo7, _dot(wqkv_ref[:, 2 * D:3 * D], wo_ref[...]))
            ln_chunk0(NLOOP + 2)
            ln_chunk0(NLOOP + 3)
            w_copy(4).start()
            x1_copy().start()
            w_copy(2).wait()
            set_w7(win7, win_ref[...].astype(F32))
            w_copy(3).wait()
            set_w7(wout7, wout_ref[...].astype(F32))
            wm7[...] = jnp.zeros(wm7.shape, U32)

        @pl.when(s == 1)
        def _():
            x1_copy().wait()
            w_copy(4).wait()
            set_w7(wm7, wm_ref[...].astype(F32))

        @pl.when(s == NT)
        def _():
            def body(j, carry):
                r = pl.multiple_of(j * 64, 64)
                for k in range(7):
                    kc_ref[k, pl.ds(r, 64), :] = kn_ref[k, pl.ds(r, 64), :]
                return carry
            lax.fori_loop(0, SH // 2 // 64, body, 0)

        def tie_head(head_u32, toks):
            return head_u32 | (functools.reduce(jnp.bitwise_or, toks) & zero)

        def zero_after(v):
            return pltpu.bitcast(pltpu.bitcast(v[:8, :128], U32) & zero, F32)

        def tied(lhs, toks):
            if not toks:
                return lhs
            head = _upk(tie_head(_pk(lhs[:16, :128]), toks))
            return jnp.concatenate(
                [jnp.concatenate([head, lhs[:16, 128:]], axis=1), lhs[16:]], axis=0)

        def tied_f32(lhs, toks):
            if not toks:
                return lhs
            head = pltpu.bitcast(tie_head(pltpu.bitcast(lhs[:8, :128], U32), toks), F32)
            return jnp.concatenate(
                [jnp.concatenate([head, lhs[:8, 128:]], axis=1), lhs[8:]], axis=0)

        def mm_units(get_lhs7, w_ref, out):
            cache = {}

            def unit(k, toks):
                if not cache:
                    cache['l'] = get_lhs7()
                out[k] = _dot(tied_f32(cache['l'][k], toks).astype(BF16), _upk(w_ref[k]))
                return out[k]
            return [functools.partial(unit, k) for k in range(7)]

        def oc(ms, r, n=RB):
            return _out_combos(*[m[r:r + n, :] for m in ms])

        def store_m_pieces(c0, head, shift, tile, ms):
            t0 = (tile % NT) * TQ - shift

            def tail():
                keep = (tile % NT) > 0
                for c in range(c0, c0 + NC):
                    m_ref[c, 0:head, :] = jnp.where(keep, m_ref[c, TQ:TQ + head, :], 0.0)
                return []

            def piece(r):
                blocks = oc(ms, r)
                row = lax.broadcasted_iota(jnp.int32, (RB, 128), 0)
                for half in range(2):
                    t = row + (t0 + half * H + r)
                    valid = (t >= 0) & (t < T)
                    for cb in range(2):
                        blk = blocks[2 * half + cb]
                        for k in range(HD // 128):
                            rr = head + half * H + r
                            m_ref[c0 + cb * (HD // 128) + k, rr:rr + RB, :] = (
                                jnp.where(valid, blk[:, k * 128:(k + 1) * 128], 0.0))
                return []
            return [tail] + [functools.partial(piece, r) for r in ROWS]

        def conv_block(ref, cw_ref, c, r, n, z=None):
            acc = None
            for d in range(KW):
                w = cw_ref[d, :, c * 128:(c + 1) * 128]
                if z is not None:
                    w = w + z
                w = jnp.concatenate([w] * (n // 8), axis=0)
                v = ref[c, PAD - 2 + d + r:PAD - 2 + d + r + n, :] * w
                acc = v if acc is None else acc + v
            return acc

        def glob_work():
            ms = [None] * 7
            units = mm_units(lambda: _lhs_f32(*[yb_ref[q] for q in range(4)]), wvo7, ms)
            return units, store_m_pieces(0, MG_H, 0, jnp.maximum(s - 1, 0), ms)

        def merge_work():
            jg = jnp.maximum(s - 1, 0)
            b = jg // NT
            base = pl.multiple_of((jg % NT) * TQ, 16)
            slot = s % 2

            def lhs_piece(c, r, z=None):
                a11 = conv_block(m_ref, cwm_ref, c, r, RB, z)
                a21 = conv_block(m_ref, cwm_ref, c, H + r, RB, z)
                a12 = conv_block(m_ref, cwm_ref, NC + c, r, RB, z)
                a22 = conv_block(m_ref, cwm_ref, NC + c, H + r, RB, z)
                for k, v in enumerate(_lhs_combos(a11, a12, a21, a22)):
                    ml7[k, r // 2:(r + RB) // 2, c * 128:(c + 1) * 128] = _pk(v)
                return []
            lhs_pieces = [functools.partial(lhs_piece, c, r) for r in ROWS for c in range(NC)]
            ms = [None] * 7

            def unit(k, toks):
                ms[k] = _dot(tied(_upk(ml7[k]), toks), _upk(wm7[k]))
                return ms[k]

            def piece(r):
                c11, c12, c21, c22 = oc(ms, r)
                for half, (lo, hi) in enumerate(((c11, c12), (c21, c22))):
                    xr = x_ref[b, pl.ds(pl.multiple_of(base + half * H + r, 16), RB), :].astype(F32)
                    ob_ref[slot, half * H + r:half * H + r + RB, :] = (
                        xr + jnp.concatenate([lo, hi], axis=1)).astype(ob_ref.dtype)
                return []
            return (lhs_pieces, [functools.partial(unit, k) for k in range(7)],
                    [functools.partial(piece, r) for r in ROWS])

        def out_copy(step, kind):
            jg = step - 1
            b = jg // NT
            j = jg % NT
            slot = step % 2
            if kind == 0:
                src_, off, n = ob_ref.at[slot, pl.ds(PX, TQ - PX), :], 0, TQ - PX
            else:
                src_, off, n = ob_ref.at[slot], pl.multiple_of(j * TQ - PX, 16), TQ
            return pltpu.make_async_copy(src_, o_hbm.at[b, pl.ds(off, n), :], osems.at[slot])

        def for_out(step, fn):
            j = (step - 1) % NT
            for kind, cond in enumerate((j == 0, j > 0)):
                @pl.when(cond)
                def _(kind=kind):
                    fn(out_copy(step, kind))

        def run(units, plan):
            outs = []
            for i, u in enumerate(units):
                toks = []
                for p, a in plan.get(i, []):
                    vals = p() if a is None else p(z=zero_after(outs[a]))
                    if vals:
                        toks.append(_token(vals))
                outs.append(u(toks))

        def spread(plan, pieces, lo, hi, lag=None):
            n = hi - lo + 1
            for j, p in enumerate(pieces):
                i = lo + (j * n) // len(pieces)
                plan.setdefault(i, []).append((p, None if lag is None else i - lag))

        def main_step():
            b = s // NT
            i = s % NT
            t0 = i * TQ
            r0 = pl.multiple_of(PAD + t0, 16)

            g_units, g_pieces = glob_work()
            qm, um = [None] * 7, [None] * 7

            def xa_rows(row0, n):
                base = pl.multiple_of(row0 // 2, 8)
                view = xa_ref.at[b, pl.ds(base, n // 2), :]
                return jnp.concatenate([_upk16(view[r // 2:r // 2 + 8, :]) for r in range(0, n, 16)], axis=0)

            lhs_cache = {}

            def xa7():
                if 'a' not in lhs_cache:
                    lhs_cache['a'] = _lhs_f32(*_split4(xa_rows(r0, TQ)))
                return lhs_cache['a']

            def q_piece(r):
                for k, v in enumerate(_lhs_combos(*oc(qm, r))):
                    q7[k, r // 2:(r + RB) // 2, :] = _pk(v)
                return []

            def ug_tail():
                keep = i > 0
                for c in range(NC):
                    u_ref[c, 0:GH, :] = jnp.where(keep, u_ref[c, TQ:TQ + GH, :], 0.0)
                    g_ref[c, 0:GH, :] = jnp.where(keep, g_ref[c, TQ:TQ + GH, :], 0.0)
                return []

            def u_piece(half, r):
                m = [None if v is None else v[r:r + RB, :] for v in um]
                v = _gelu(_out_block(2 * half, m))
                rr = GH + half * H + r
                for c in range(NC):
                    u_ref[c, rr:rr + RB, :] = v[:, c * 128:(c + 1) * 128]
                return []

            def gt_piece(half, r, z=None):
                m = [None if v is None else v[r:r + RB, :] for v in um]
                pre = _out_block(2 * half + 1, m)
                if z is not None:
                    pre = pre + jnp.concatenate([jnp.concatenate([z, z], axis=0)] * NC, axis=1)
                g = _ln(_gelu(pre))
                valid = (lax.broadcasted_iota(jnp.int32, (RB, 128), 0) + (t0 + half * H + r)) < T
                rr = GH + half * H + r
                for c in range(NC):
                    g_ref[c, rr:rr + RB, :] = jnp.where(valid, g[:, c * 128:(c + 1) * 128], 0.0)
                return []

            def kop(k, sl):
                return _upk(kc_ref[k, sl.start // 2:sl.stop // 2, :])

            km = [[None] * 7 for _ in range(NCH)]

            KORD = [1, 3, 2, 4, 0, 5, 6]

            def k_units(c):
                sl = slice(c * W, (c + 1) * W)

                def unit(k, toks):
                    km[c][k] = _dot_nt(tied(_upk(q7[k]), toks), kop(k, sl))
                    return km[c][k]
                return [functools.partial(unit, k) for k in KORD]

            stat = {}

            def k_piece(c, blk, r):
                sl = slice(c * W, (c + 1) * W)
                m = [None if v is None else v[r:r + RB, :] for v in km[c]]
                v = _out_block(blk, m)
                if blk in (1, 3) and SH + (c + 1) * W > T:
                    col = lax.broadcasted_iota(jnp.int32, (RB, W), 1)
                    v = jnp.where(col < (T - SH - c * W), v, NEG)
                s_ref[blk + zs, r:r + RB, sl] = v
                tiles = [v[:, k * 128:(k + 1) * 128] for k in range(W // 128)]
                cm = functools.reduce(jnp.maximum, tiles)
                prev = stat.get((blk // 2, r))
                if prev is not None:
                    cm = jnp.maximum(cm, prev[0])
                l = functools.reduce(jnp.add, [jnp.exp2(t - cm) for t in tiles])
                if prev is not None:
                    l = l + prev[1] * jnp.exp2(prev[0] - cm)
                stat[blk // 2, r] = (cm, l)
                return [l]

            def k_pieces(c, blk):
                return [functools.partial(k_piece, c, blk, r) for r in ROWS]

            def fin(h):
                ms = jnp.concatenate([stat[h, r][0] for r in ROWS], axis=0)
                ls = jnp.concatenate([stat[h, r][1] for r in ROWS], axis=0)
                m = jnp.max(ms, axis=1, keepdims=True)
                return m + jnp.log2(jnp.sum(ls * jnp.exp2(ms - m), axis=1, keepdims=True))

            lb = jnp.where((s >= 1) & (s < NT), 1, 0)
            db = jnp.where(s < NT, 1, 0)
            lc = jnp.where(s < NT, jnp.maximum(s - 1, 0), (s - NT) % NLC)
            ln_pieces = [functools.partial(ln_rows, kn_ref, lb, db, lc, r) for r in range(0, LC, RB)]

            n = [None] * 7
            tmap = [0, 6, 1, 4, 5, 3, 2]
            off = []

            def fin_piece():
                off.extend([fin(0), fin(1)])
                return [jnp.broadcast_to(o, (H, 128)) for o in off]

            def p_units(c):
                sl = slice(c * W, (c + 1) * W)
                cache = {}

                def lhs(k):
                    if not cache:
                        cache['p'] = [jnp.exp2(s_ref[idx + zs, :, sl] - off[idx // 2]) for idx in range(4)]
                    p11, p12, p21, p22 = cache['p']
                    return [lambda: p11 + p22, lambda: p11, lambda: p21 - p22, lambda: p12 - p11,
                            lambda: p22, lambda: p11 + p21, lambda: p12 + p22][k]()

                def unit(k, toks):
                    r = _dot(tied_f32(lhs(k), toks).astype(BF16), kop(tmap[k], sl))
                    n[k] = r if n[k] is None else n[k] + r
                    return r
                return [functools.partial(unit, k) for k in (1, 4, 0, 3, 2, 5, 6)]

            def z_piece(c, r):
                vals = []
                for cc in (c, c + NC // 2):
                    for half in range(2):
                        rr = half * H + r
                        gc = conv_block(g_ref, cwc_ref, cc, rr, RB)
                        vals.append(u_ref[cc, PAD + rr:PAD + rr + RB, :] * gc)
                a11, a21, a12, a22 = vals
                for k, v in enumerate(_lhs_combos(a11, a12, a21, a22)):
                    z7[k, r // 2:(r + RB) // 2, c * 128:(c + 1) * 128] = _pk(v)
                return [a11 + a22, a12 + a21]
            z_pieces = [functools.partial(z_piece, c, r) for r in ROWS for c in range(NC // 2)]
            lm = [None] * 7

            def l_unit(k, toks):
                lm[k] = _dot(tied(_upk(z7[k]), toks), _upk(wout7[k]))
                return lm[k]

            def y_piece(r):
                n1, n2, n3, n4, n5, n6, n7 = [v[r:r + RB, :] for v in n]
                yb_ref[0, r:r + RB, :] = n1 + n4 - n5 + n7
                yb_ref[1, r:r + RB, :] = n2 + n4
                yb_ref[2, r:r + RB, :] = n3 + n5
                yb_ref[3, r:r + RB, :] = n1 - n2 + n3 + n6
                return []

            mc_pieces, mg_units, mg_pieces = merge_work()
            ut_units = mm_units(xa7, win7, um)
            units = (g_units + mm_units(xa7, a7, qm) + [ut_units[k] for k in KORD]
                     + k_units(0) + k_units(1) + k_units(2) + k_units(3) + mg_units
                     + p_units(0) + p_units(1) + p_units(2) + p_units(3)
                     + [functools.partial(l_unit, k) for k in range(7)])
            G, Q, UT, K0, K1, K2, K3, MG, P0, L = 0, 7, 14, 21, 28, 35, 42, 49, 56, 84
            plan = {}
            plan.setdefault(G + 1, []).append((ug_tail, None))
            spread(plan, g_pieces, Q + 2, UT + 1)
            spread(plan, [functools.partial(q_piece, r) for r in ROWS], UT + 1, UT + 5)
            spread(plan, [functools.partial(u_piece, 1, r) for r in ROWS], UT + 4, UT + 6)
            spread(plan, [functools.partial(u_piece, 0, r) for r in ROWS], K0 + 2, K0 + 4)
            spread(plan, [functools.partial(gt_piece, 0, r) for r in ROWS], K0 + 3, K0 + 5, lag=3)
            spread(plan, [functools.partial(gt_piece, 1, r) for r in ROWS], K0 + 6, K0 + 13, lag=3)
            spread(plan, mc_pieces, K0 + 3, MG, lag=3)
            for c in range(NCH):
                u0 = K0 + 7 * c
                spread(plan, k_pieces(c, 2), u0 + 3, u0 + 4)
                spread(plan, k_pieces(c, 1), u0 + 5, u0 + 6)
                spread(plan, k_pieces(c, 3), u0 + 8, u0 + 9)
                spread(plan, k_pieces(c, 0), u0 + 9, u0 + 10)
            plan.setdefault(MG + 4, []).append((fin_piece, None))
            spread(plan, mg_pieces, P0 + 2, P0 + 8)
            for j, p in enumerate(ln_pieces):
                plan.setdefault(L, []).append((p, P0 + (j * 24) // len(ln_pieces)))
            spread(plan, z_pieces, P0 + 7, P0 + 27)
            spread(plan, [functools.partial(y_piece, r) for r in ROWS], L + 2, L + 6)
            run(units, plan)
            for p in store_m_pieces(NC, ML_H, PAD, s, lm):
                p()

        @pl.when(s >= 3)
        def _():
            for_out(s - 2, lambda cp: cp.wait())

        @pl.when(s < NTT)
        def _():
            main_step()

        @pl.when(s >= NTT)
        def _():
            g_units, g_pieces = glob_work()
            run(g_units, {})
            for p in g_pieces:
                p()
            mc_pieces, mg_units, mg_pieces = merge_work()
            for p in mc_pieces:
                p()
            run(mg_units, {})
            for p in mg_pieces:
                p()

        @pl.when(s >= 1)
        def _():
            for_out(s, lambda cp: cp.start())

        @pl.when(s == NSTEPS - 1)
        def _():
            for_out(s - 1, lambda cp: cp.wait())
            for_out(s, lambda cp: cp.wait())

    anyspec = pl.BlockSpec(memory_space=pl.ANY)

    def full(shape):
        return pl.BlockSpec(shape, lambda s: (0,) * len(shape))

    return pl.pallas_call(
        kernel,
        grid=(NSTEPS,),
        in_specs=[anyspec, anyspec, anyspec, anyspec, full(dw_csgu.shape), anyspec,
                  full(dw_merge.shape), anyspec],
        out_specs=anyspec,
        out_shape=jax.ShapeDtypeStruct((B, T, D), x.dtype),
        scratch_shapes=[
            pltpu.VMEM((2, TQ, D), x.dtype),
            pltpu.VMEM((B, PX + S, D), BF16),
            pltpu.VMEM((D, 3 * D), BF16),
            pltpu.VMEM((D, D), BF16),
            pltpu.VMEM((D, 2 * D), BF16),
            pltpu.VMEM((D, D), BF16),
            pltpu.VMEM((2 * D, D), BF16),
            pltpu.VMEM((B, XR // 2, D), U32),
            pltpu.VMEM((7, SH // 2, HD), U32),
            pltpu.VMEM((7, SH // 2, HD), U32),
            pltpu.VMEM((7, HD // 2, HD), U32),
            pltpu.VMEM((7, HD // 2, D), U32),
            pltpu.VMEM((7, HD // 2, HD), U32),
            pltpu.VMEM((7, HD // 2, HD), U32),
            pltpu.VMEM((7, D // 2, HD), U32),
            pltpu.VMEM((KW, 8, D), F32),
            pltpu.VMEM((KW, 8, 2 * D), F32),
            pltpu.VMEM((4, H, SH), F32),
            pltpu.VMEM((4, H, HD), F32),
            pltpu.VMEM((7, H // 2, HD), U32),
            pltpu.VMEM((7, H // 2, HD), U32),
            pltpu.VMEM((7, H // 2, D), U32),
            pltpu.VMEM((NC, GH + TQ, 128), F32),
            pltpu.VMEM((NC, GH + TQ, 128), F32),
            pltpu.VMEM((2 * NC, MR, 128), F32),
            pltpu.SemaphoreType.DMA((6,)),
            pltpu.SemaphoreType.DMA((2 * NLC,)),
            pltpu.SemaphoreType.DMA((2,)),
        ],
        compiler_params=pltpu.CompilerParams(
            dimension_semantics=("arbitrary",), vmem_limit_bytes=110 * 1024 * 1024),
    )(x, w_qkv, w_att_out, w_mlp_in, dw_csgu, w_mlp_out, dw_merge, w_merge)
```
